```python
import jax
import jax.numpy as jnp

def _softmax(x, axis=-1):
    return jax.nn.softmax(x, axis=axis)

def _gelu(x):
    return jax.nn.gelu(x, approximate=True)

def _silu(x):
    return jax.nn.silu(x)

def _sigmoid(x):
    return jax.nn.sigmoid(x)

def _layernorm(x, axis=-1, eps=1e-05):
    m = jnp.mean(x, axis=axis, keepdims=True)
    v = jnp.var(x, axis=axis, keepdims=True)
    return (x - m) / jnp.sqrt(v + eps)

def _scatter_add(tgt, idx, src, axis=0):
    return tgt.at[idx].add(src)

def _segment_sum(src, seg, n):
    return jax.ops.segment_sum(src, seg, n)

class _Rng:

    def __init__(self, key):
        self._k = key

    def _next(self):
        self._k, sub = jax.random.split(self._k)
        return sub

    def normal(self, shape):
        return jax.random.normal(self._next(), shape, dtype=jnp.bfloat16)

    def randint(self, lo, hi, shape):
        return jax.random.randint(self._next(), shape, lo, hi, dtype=jnp.int32)

    def uniform(self, shape, lo=0.0, hi=1.0):
        return jax.random.uniform(self._next(), shape, jnp.bfloat16, lo, hi)

    def permutation(self, n):
        return jax.random.permutation(self._next(), n)
kernel_name = 'sequential_preLN__memory_aug_recurrent_mem_tr__mixer_s_mlp__prompt'

def setup_inputs():
    _rng = _Rng(jax.random.key(int.from_bytes(__import__("os").urandom(4), "little")))
    _w = lambda a: (lambda t: t.astype(jnp.bfloat16) if jnp.issubdtype(t.dtype, jnp.floating) else t)(jnp.asarray(a))

    def _A_setup():
        B, S, Dm = (1, 2048, 1024)
        H, Dh = (32, 128)
        M, seg = (8, 32)
        seg = min(seg, S)
        S = S // seg * seg
        return {'x': _w((lambda *s: _rng.normal(s) * 0.05)(B, S, Dm)), 'mem0': _w((lambda *s: _rng.normal(s) * 0.05)(B, M, Dm)), 'Wq': _w((lambda *s: _rng.normal(s) * 0.05)(Dm, H, Dh) * Dm ** (-0.5)), 'Wk': _w((lambda *s: _rng.normal(s) * 0.05)(Dm, H, Dh) * Dm ** (-0.5)), 'Wv': _w((lambda *s: _rng.normal(s) * 0.05)(Dm, H, Dh) * Dm ** (-0.5)), 'Wo': _w((lambda *s: _rng.normal(s) * 0.05)(H, Dh, Dm) * (H * Dh) ** (-0.5)), 'seg_len': seg}
    _A_in = _A_setup()

    def _B_setup():
        B, S, D, F = (1, 2048, 1024, 3584)
        return {'x': _w((lambda *s: _rng.normal(s) * 0.05)(B, S, D)), 'w1': _w((lambda *s: _rng.normal(s) * 0.05)(D, D) * D ** (-0.5)), 'w2': _w((lambda *s: _rng.normal(s) * 0.05)(D, D) * D ** (-0.5)), 'w3': _w((lambda *s: _rng.normal(s) * 0.05)(D, F) * D ** (-0.5)), 'w4': _w((lambda *s: _rng.normal(s) * 0.05)(F, D) * F ** (-0.5))}
    _B_in = _B_setup()
    return {'A_x': _A_in['x'], 'A_mem0': _A_in['mem0'], 'A_Wq': _A_in['Wq'], 'A_Wk': _A_in['Wk'], 'A_Wv': _A_in['Wv'], 'A_Wo': _A_in['Wo'], 'A_seg_len': _A_in['seg_len'], 'B_x': _B_in['x'], 'B_w1': _B_in['w1'], 'B_w2': _B_in['w2'], 'B_w3': _B_in['w3'], 'B_w4': _B_in['w4']}

def reference(A_x, A_mem0, A_Wq, A_Wk, A_Wv, A_Wo, A_seg_len, B_x, B_w1, B_w2, B_w3, B_w4):

    def _A_ref(x, mem0, Wq, Wk, Wv, Wo, seg_len):
        B, S, Dm = x.shape
        H, Dh = (Wq.shape[1], Wq.shape[2])
        M = mem0.shape[1]
        scale = Dh ** (-0.5)
        n_seg = S // seg_len
        L = M + seg_len
        idx = jnp.arange(L)
        mask = (idx[:, None] < M) | (idx[:, None] >= idx[None, :])
        mem = mem0
        outs = []
        for s in range(n_seg):
            xs = x[:, s * seg_len:(s + 1) * seg_len, :].copy()
            h = jnp.concatenate([mem, xs], axis=1)
            q = jnp.einsum('btd,dhe->bhte', h, Wq)
            k = jnp.einsum('btd,dhe->bhte', h, Wk)
            v = jnp.einsum('btd,dhe->bhte', h, Wv)
            scores = jnp.einsum('bhqe,bhke->bhqk', q, k) * scale
            scores = jnp.where(mask[None, None], scores, -1000000000.0)
            p = _softmax(scores, axis=-1)
            o = jnp.einsum('bhqk,bhke->bhqe', p, v)
            o = jnp.einsum('bhte,hed->btd', o, Wo)
            mem = o[:, :M, :].copy()
            outs.append(o[:, M:, :])
        return jnp.concatenate(outs, axis=1)

    def _B_ref(x, w1, w2, w3, w4):
        B, S, D = x.shape
        h = _gelu(_layernorm(x, axis=-1) @ w1)
        c = D // 4
        g0 = jnp.pad(h[:, :, 0 * c:1 * c], ((0, 0), (1, 0), (0, 0)))[:, :S, :]
        g1 = jnp.pad(h[:, :, 1 * c:2 * c], ((0, 0), (0, 1), (0, 0)))[:, 1:, :]
        g2 = jnp.pad(h[:, :, 2 * c:3 * c], ((0, 0), (2, 0), (0, 0)))[:, :S, :]
        g3 = jnp.pad(h[:, :, 3 * c:], ((0, 0), (0, 2), (0, 0)))[:, 2:, :]
        hs = jnp.concatenate([g0, g1, g2, g3], axis=-1) @ w2
        x1 = x + hs
        h2 = _gelu(_layernorm(x1, axis=-1) @ w3) @ w4
        return x1 + h2
    x = A_x
    h = x + _A_ref(_layernorm(x, axis=-1), A_mem0, A_Wq, A_Wk, A_Wv, A_Wo, A_seg_len)
    h2 = h + _B_ref(_layernorm(h, axis=-1), B_w1, B_w2, B_w3, B_w4)
    return h2
```

```python
import functools

import jax
import jax.numpy as jnp
from jax import lax
from jax.experimental import pallas as pl
from jax.experimental.pallas import tpu as pltpu

bf16, f32, u32 = jnp.bfloat16, jnp.float32, jnp.uint32

LN_EPS = 1e-5
NX = 8
HG = 8
RB = 256
FC = 512

S_XE, S_XF, S_LAND, S_WO, S_W1, S_W2, S_W3, S_W4, S_OUT = 0, 1, 2, 5, 6, 7, 8, 9, 10
N_SEMS = 12


def _pk(x):
    return pltpu.bitcast(x, u32)


def _upk(x):
    return pltpu.bitcast(x, bf16)


def _dot(a, b):
    return jnp.dot(a, b, preferred_element_type=f32)


def _ln(x):
    m = jnp.mean(x, axis=-1, keepdims=True)
    xc = x - m
    v = jnp.mean(xc * xc, axis=-1, keepdims=True)
    return xc * lax.rsqrt(v + LN_EPS)


def _gelu(x):
    return 0.5 * x * (1.0 + jnp.tanh(0.7978845608028654 * (x + 0.044715 * (x * x * x))))


def _repack(src, dst, rows, blk):
    for r in range(0, rows, blk):
        dst[r // 2:(r + blk) // 2, :] = _pk(src[r:r + blk, :])


def _kernel(x_hbm, mem0_ref, wq_hbm, wk_hbm, wv_hbm, wo_hbm, w1_hbm, w2_hbm, w3_hbm, w4_hbm,
            out_hbm,
            x_s, h_s, oex_s, wo_p, w1_l, w2_l, w3_l, w4_l, sems,
            *, NSEG, SEG, D, H, E, M, F):
    S = NSEG * SEG
    NF = SEG - NX
    NR = M + NF
    L = M + SEG
    LP = L + 8
    HE = H * E
    NG = H // HG
    w_hbm = (wq_hbm, wk_hbm, wv_hbm)

    def cp_xe():
        return pltpu.make_async_copy(x_hbm.at[:, NF:SEG, :], x_s.at[:, NF:SEG, :], sems.at[S_XE])

    def cp_xf():
        return pltpu.make_async_copy(x_hbm.at[:, 0:NF, :], x_s.at[:, 0:NF, :], sems.at[S_XF])

    def cp_wo(wo_l):
        return pltpu.make_async_copy(wo_hbm, wo_l, sems.at[S_WO])

    b_copies = [
        pltpu.make_async_copy(w1_hbm, w1_l, sems.at[S_W1]),
        pltpu.make_async_copy(w2_hbm, w2_l, sems.at[S_W2]),
        pltpu.make_async_copy(w3_hbm, w3_l, sems.at[S_W3]),
        pltpu.make_async_copy(w4_hbm, w4_l, sems.at[S_W4]),
    ]

    def phase_a(wqkv_p, wo_l, land, stage, xe_p, xln_s, qkvx_s):
        def cp_chunk(w, g):
            g0 = pl.multiple_of(g * HG, HG)
            return pltpu.make_async_copy(w_hbm[w].at[:, pl.ds(g0, HG), :], land.at[w],
                                         sems.at[S_LAND + w])

        def relayout(w, g):
            db = 64
            for d0 in range(0, D, db):
                stage[d0 * 4:(d0 + db) * 4, :] = _pk(land[w, d0:d0 + db].reshape(db * HG, E))
            col0 = w * HE + g * (HG * E)
            for p in range(HG // 2):
                for d0 in range(0, D, 128):
                    u = stage[pl.ds(d0 * 4 + p, 128, stride=4), :]
                    lo = pltpu.bitcast(u << 16, f32).astype(bf16)
                    hi = pltpu.bitcast(u & jnp.uint32(0xFFFF0000), f32).astype(bf16)
                    c_lo = pl.multiple_of(col0 + (2 * p) * E, E)
                    c_hi = pl.multiple_of(col0 + (2 * p + 1) * E, E)
                    wqkv_p[d0 // 2:d0 // 2 + 64, pl.ds(c_lo, E)] = _pk(lo)
                    wqkv_p[d0 // 2:d0 // 2 + 64, pl.ds(c_hi, E)] = _pk(hi)

        def proj_extra(w, g):
            col0 = w * HE + g * (HG * E)
            nb = 512
            for mb in range(NSEG * NX // 256):
                a = _upk(xe_p[mb * 128:(mb + 1) * 128, :])
                for nc in range(HG * E // nb):
                    c = pl.multiple_of(col0 + nc * nb, nb)
                    r = _dot(a, _upk(wqkv_p[:, pl.ds(c, nb)]))
                    qkvx_s[mb * 256:(mb + 1) * 256, pl.ds(c, nb)] = r.astype(bf16)

        cp_xe().start()
        for w in range(3):
            cp_chunk(w, 0).start()
        cp_xf().start()

        cp_xe().wait()
        sb = 16
        for s0 in range(0, NSEG, sb):
            xe = x_s[s0:s0 + sb, NF:SEG, :].astype(f32).reshape(sb * NX, D)
            xe_p[s0 * NX // 2:(s0 + sb) * NX // 2, :] = _pk(_ln(xe).astype(bf16))
        cp_chunk(0, 0).wait()
        relayout(0, 0)
        cp_chunk(0, 1).start()

        gseg = NSEG // NG

        def chunk_body(g, carry):
            nxt = jnp.minimum(g + 1, NG - 1)
            cp_chunk(1, g).wait()
            relayout(1, g)
            proj_extra(0, g)

            @pl.when(g < NG - 1)
            def _():
                cp_chunk(1, g + 1).start()

            cp_chunk(2, g).wait()
            relayout(2, g)
            proj_extra(1, g)

            @pl.when(g < NG - 1)
            def _():
                cp_chunk(2, g + 1).start()
                cp_chunk(0, g + 1).wait()

            @pl.when(g == 0)
            def _():
                cp_xf().wait()
                cp_wo(wo_l).start()

            relayout(0, nxt)
            proj_extra(2, g)
            s0 = pl.multiple_of(g * gseg, gseg)
            for j in range(0, gseg, 4):
                xf = x_s[pl.ds(s0 + j, 4), 0:NF, :].astype(f32)
                xln_s[pl.ds(s0 + j, 4)] = _ln(xf).astype(bf16)

            @pl.when(g < NG - 2)
            def _():
                cp_chunk(0, g + 2).start()

            return carry

        lax.fori_loop(0, NG, chunk_body, 0)

        for c in b_copies:
            c.start()
        cp_wo(wo_l).wait()
        _repack(wo_l, wo_p, HE, 256)

        scale = E ** -0.5
        row = lax.broadcasted_iota(jnp.int32, (L, LP), 0)
        col = lax.broadcasted_iota(jnp.int32, (L, LP), 1)
        allowed = (row < M) | (row >= col)
        valid = col < L
        zpad = jnp.zeros((LP - L, E), bf16)
        DS, DP = 1, 4
        WO_SPLIT = 4
        hs = H // WO_SPLIT

        def step(s, mem):
            e0 = pl.multiple_of(s * NX, NX)
            xs = xln_s[s].astype(f32)
            lhs = jnp.concatenate([mem, xs], axis=0).astype(bf16)
            qs, ks, vs, ps, outs, ys = {}, {}, {}, {}, {}, []

            def proj(h):
                qs[h] = _dot(lhs, _upk(wqkv_p[:, h * E:(h + 1) * E]))
                ks[h] = _dot(lhs, _upk(wqkv_p[:, HE + h * E:HE + (h + 1) * E]))
                vs[h] = _dot(lhs, _upk(wqkv_p[:, 2 * HE + h * E:2 * HE + (h + 1) * E]))

            def scores(h):
                qx = qkvx_s[pl.ds(e0, NX), h * E:(h + 1) * E]
                kx = qkvx_s[pl.ds(e0, NX), HE + h * E:HE + (h + 1) * E]
                q = jnp.concatenate([qs[h].astype(bf16), qx], axis=0)
                k = jnp.concatenate([ks[h].astype(bf16), kx, zpad], axis=0)
                sc = lax.dot_general(q, k, (((1,), (1,)), ((), ())),
                                     preferred_element_type=f32) * scale
                sc = jnp.where(allowed, sc, -1e9)
                sc = jnp.where(valid, sc, -jnp.inf)
                m = jnp.max(sc, axis=-1, keepdims=True)
                p = jnp.exp(sc - m)
                l = jnp.sum(p, axis=-1, keepdims=True)
                r = pl.reciprocal(l, approx=True)
                r = r * (2.0 - l * r)
                ps[h] = (p * r).astype(bf16)

            def pv(h):
                vx = qkvx_s[pl.ds(e0, NX), 2 * HE + h * E:2 * HE + (h + 1) * E]
                v = jnp.concatenate([vs[h].astype(bf16), vx, zpad], axis=0)
                o = _dot(ps[h], v)
                oex_s[pl.ds(e0, NX), h * E:(h + 1) * E] = o[NR:L].astype(bf16)
                outs[h] = o[0:NR].astype(bf16)

            def wo(j):
                oj = jnp.concatenate([outs[h] for h in range(j * hs, (j + 1) * hs)], axis=1)
                ys.append(_dot(oj, _upk(wo_p[j * hs * E // 2:(j + 1) * hs * E // 2, :])))

            for t in range(H):
                proj(t)
                if t >= DS:
                    scores(t - DS)
                if t >= DP:
                    pv(t - DP)
            wo(0)
            scores(H - 1)
            pv(H - 4)
            pv(H - 3)
            wo(1)
            pv(H - 2)
            wo(2)
            pv(H - 1)
            wo(3)
            y = (ys[0] + ys[1]) + (ys[2] + ys[3])
            h_s[s, 0:NF, :] = x_s[s, 0:NF, :].astype(f32) + y[M:]
            return y[:M].astype(bf16).astype(f32)

        lax.fori_loop(0, NSEG, step, mem0_ref[...].astype(f32))

    pl.run_scoped(
        phase_a,
        pltpu.VMEM((D // 2, 3 * HE), u32),
        pltpu.VMEM((HE, D), bf16),
        pltpu.VMEM((3, D, HG, E), bf16),
        pltpu.VMEM((D * HG // 2, E), u32),
        pltpu.VMEM((NSEG * NX // 2, D), u32),
        pltpu.VMEM((NSEG, NF, D), bf16),
        pltpu.VMEM((NSEG * NX, 3 * HE), bf16),
    )

    NB = S // RB
    bseg = RB // SEG
    cq = D // 4

    def phase_b(w1_p, w2_p, w3_p, w4_p, g_s, a_s, r_s, u_s, o_st):
        for c in b_copies:
            c.wait()
        _repack(w1_l, w1_p, D, 256)
        _repack(w2_l, w2_p, D, 256)
        _repack(w3_l, w3_p, D, 64)
        _repack(w4_l, w4_p, F, 256)
        g_s[0:8, :] = jnp.zeros((8, D), f32)
        g_s[S + 8:S + 16, :] = jnp.zeros((8, D), f32)

        def b1_body(i, carry):
            s0 = pl.multiple_of(i * bseg, bseg)
            e0 = pl.multiple_of(i * (bseg * NX), bseg * NX)
            yx = _dot(oex_s[pl.ds(e0, bseg * NX), :], _upk(wo_p[...]))
            xe = x_s[pl.ds(s0, bseg), NF:SEG, :].astype(f32)
            h_s[pl.ds(s0, bseg), NF:SEG, :] = xe + yx.reshape(bseg, NX, D)
            hb = h_s[pl.ds(s0, bseg)].reshape(RB, D)
            a = _ln(_ln(hb)).astype(bf16)
            r0 = pl.multiple_of(i * RB + 8, 8)
            for c in range(4):
                g = _gelu(_dot(a, _upk(w1_p[:, c * cq:(c + 1) * cq])))
                g_s[pl.ds(r0, RB), c * cq:(c + 1) * cq] = g
            return carry

        lax.fori_loop(0, NB, b1_body, 0)

        def cp_out(i, slot):
            r0 = pl.multiple_of(i * RB, RB)
            return pltpu.make_async_copy(o_st.at[slot], out_hbm.at[pl.ds(r0, RB), :],
                                         sems.at[S_OUT + slot])

        def mix(i):
            r0 = pl.multiple_of(i * RB, RB)
            s0 = pl.multiple_of(i * bseg, bseg)
            g0 = g_s[pl.ds(r0, RB + 16), 0 * cq:1 * cq][7:7 + RB]
            g1 = g_s[pl.ds(r0, RB + 16), 1 * cq:2 * cq][9:9 + RB]
            g2 = g_s[pl.ds(r0, RB + 16), 2 * cq:3 * cq][6:6 + RB]
            g3 = g_s[pl.ds(r0, RB + 16), 3 * cq:4 * cq][10:10 + RB]
            gs = jnp.concatenate([g0, g1, g2, g3], axis=1).astype(bf16)
            hsft = _dot(gs, _upk(w2_p[...]))
            hb = h_s[pl.ds(s0, bseg)].reshape(RB, D)
            x1 = _ln(hb) + hsft
            a_s[...] = _pk(_ln(x1).astype(bf16))
            r_s[i % 2] = hb + x1

        mix(0)

        def b2_body(i, carry):
            slot = i % 2

            @pl.when(i >= 2)
            def _():
                cp_out(i - 2, slot).wait()

            a = _upk(a_s[...])
            for c in range(F // FC):
                u = _dot(a, _upk(w3_p[:, c * FC:(c + 1) * FC]))
                u_s[:, c * FC:(c + 1) * FC] = _pk(_gelu(u).astype(bf16))
            mix(jnp.minimum(i + 1, NB - 1))
            y = _dot(_upk(u_s[...]), _upk(w4_p[...]))
            o_st[slot] = (r_s[slot] + y).astype(bf16)
            cp_out(i, slot).start()
            return carry

        lax.fori_loop(0, NB, b2_body, 0)
        cp_out(NB - 2, (NB - 2) % 2).wait()
        cp_out(NB - 1, (NB - 1) % 2).wait()

    pl.run_scoped(
        phase_b,
        pltpu.VMEM((D // 2, D), u32),
        pltpu.VMEM((D // 2, D), u32),
        pltpu.VMEM((D // 2, F), u32),
        pltpu.VMEM((F // 2, D), u32),
        pltpu.VMEM((S + 16, D), f32),
        pltpu.VMEM((RB // 2, D), u32),
        pltpu.VMEM((2, RB, D), f32),
        pltpu.VMEM((RB // 2, F), u32),
        pltpu.VMEM((2, RB, D), bf16),
    )


@functools.partial(jax.jit, static_argnames=("A_seg_len",))
def pallas_sequential_preLN__memory_aug_recurrent_mem_tr__mixer_s_mlp__prompt_kernel(
    A_x: jax.Array,
    A_mem0: jax.Array,
    A_Wq: jax.Array,
    A_Wk: jax.Array,
    A_Wv: jax.Array,
    A_Wo: jax.Array,
    A_seg_len: int,
    B_x: jax.Array,
    B_w1: jax.Array,
    B_w2: jax.Array,
    B_w3: jax.Array,
    B_w4: jax.Array,
):
    del B_x
    B, S, D = A_x.shape
    _, H, E = A_Wq.shape
    M = A_mem0.shape[1]
    F = B_w3.shape[1]
    SEG = int(A_seg_len)
    NSEG = S // SEG
    assert B == 1 and M == 8 and SEG == 32 and E == 128 and S == NSEG * SEG
    assert H % HG == 0 and S % RB == 0 and F % FC == 0 and D % 256 == 0
    assert (NSEG * NX) % 256 == 0 and NSEG % (4 * (H // HG)) == 0 and NSEG % 16 == 0

    hbm = pl.BlockSpec(memory_space=pl.ANY)
    kernel = functools.partial(_kernel, NSEG=NSEG, SEG=SEG, D=D, H=H, E=E, M=M, F=F)
    out = pl.pallas_call(
        kernel,
        out_shape=jax.ShapeDtypeStruct((S, D), A_x.dtype),
        in_specs=[hbm, pl.BlockSpec(memory_space=pltpu.VMEM)] + [hbm] * 8,
        out_specs=hbm,
        scratch_shapes=[
            pltpu.VMEM((NSEG, SEG, D), bf16),
            pltpu.VMEM((NSEG, SEG, D), f32),
            pltpu.VMEM((NSEG * NX, H * E), bf16),
            pltpu.VMEM((H * E // 2, D), u32),
            pltpu.VMEM((D, D), bf16),
            pltpu.VMEM((D, D), bf16),
            pltpu.VMEM((D, F), bf16),
            pltpu.VMEM((F, D), bf16),
            pltpu.SemaphoreType.DMA((N_SEMS,)),
        ],
        compiler_params=pltpu.CompilerParams(vmem_limit_bytes=124 * 1024 * 1024),
        name="rmt_mixer",
    )(
        A_x.reshape(NSEG, SEG, D),
        A_mem0.reshape(M, D),
        A_Wq, A_Wk, A_Wv,
        A_Wo.reshape(H * E, D),
        B_w1, B_w2, B_w3, B_w4,
    )
    return out.reshape(B, S, D)
```

```python
import functools

import jax
import jax.numpy as jnp
from jax import lax
from jax.experimental import pallas as pl
from jax.experimental.pallas import tpu as pltpu

bf16, f32, u32 = jnp.bfloat16, jnp.float32, jnp.uint32

LN_EPS = 1e-5
NX = 8
HG = 8
RB = 128
FC = 512

S_XE, S_XF, S_LAND, S_WO, S_MEM, S_B0, S_B1, S_OUT = 0, 1, 2, 5, 6, 7, 11, 15
N_SEMS = 17


def _pk(x):
    return pltpu.bitcast(x, u32)


def _upk(x):
    return pltpu.bitcast(x, bf16)


def _dot(a, b):
    return jnp.dot(a, b, preferred_element_type=f32)


def _ln(x):
    m = jnp.mean(x, axis=-1, keepdims=True)
    xc = x - m
    v = jnp.mean(xc * xc, axis=-1, keepdims=True)
    return xc * lax.rsqrt(v + LN_EPS)


def _ln2(x):
    m = jnp.mean(x, axis=-1, keepdims=True)
    xc = x - m
    v = jnp.mean(xc * xc, axis=-1, keepdims=True)
    r = lax.rsqrt(v + LN_EPS)
    return xc * (r * lax.rsqrt(v * (r * r) + LN_EPS))


def _gelu(x):
    return 0.5 * x * (1.0 + jnp.tanh(0.7978845608028654 * (x + 0.044715 * (x * x * x))))


def _repack(src, dst, rows, blk):
    for r in range(0, rows, blk):
        dst[r // 2:(r + blk) // 2, :] = _pk(src[r:r + blk, :])


def _kernel(x_hbm, mem0_hbm, wq_hbm, wk_hbm, wv_hbm, wo_hbm, w1_hbm, w2_hbm, w3_hbm, w4_hbm,
            out_hbm,
            x_s, h_s, mem0_s, w1_l, w2_l, w3_l, w4_l, w1_p, w2_p, w3_p, w4_p, sems,
            *, NSEG, SEG, D, H, E, M, F):
    S = NSEG * SEG
    NF = SEG - NX
    NR = M + NF
    L = M + SEG
    LP = L + 8
    HE = H * E
    NG = H // HG
    w_hbm = (wq_hbm, wk_hbm, wv_hbm)

    def cp_xe():
        return pltpu.make_async_copy(x_hbm.at[:, NF:SEG, :], x_s.at[:, NF:SEG, :], sems.at[S_XE])

    NPAIR = NSEG // 2
    b_hbm = (w1_hbm, w2_hbm, w3_hbm, w4_hbm)
    b_land = (w1_l, w2_l, w3_l, w4_l)
    b_pack = (w1_p, w2_p, w3_p, w4_p)
    b_rows = tuple(r.shape[0] // NPAIR for r in b_hbm)

    def cp_b_first():
        return [pltpu.make_async_copy(h.at[0:n], l.at[0:n], sems.at[S_B0 + j])
                for j, (h, l, n) in enumerate(zip(b_hbm, b_land, b_rows))]

    def cp_b_rest():
        return [pltpu.make_async_copy(h.at[n:], l.at[n:], sems.at[S_B1 + j])
                for j, (h, l, n) in enumerate(zip(b_hbm, b_land, b_rows))]

    def cp_mem():
        return pltpu.make_async_copy(mem0_hbm, mem0_s, sems.at[S_MEM])

    def phase_a(wq_p, wk_p, wv_p, wo_l, wo_p, land, stage, xe_p, xn_p, qkvx_s, oex_s):
        w_p = (wq_p, wk_p, wv_p)
        CW = HG * E

        def cp_chunk(w, g):
            g0 = pl.multiple_of(g * HG, HG)
            return pltpu.make_async_copy(w_hbm[w].at[:, pl.ds(g0, HG), :], land.at[w],
                                         sems.at[S_LAND + w])

        def cp_wo(g):
            r0 = pl.multiple_of(g * CW, CW)
            return pltpu.make_async_copy(wo_hbm.at[pl.ds(r0, CW), :], wo_l, sems.at[S_WO])

        def relayout(w, dst, col0):
            db = 64
            for d0 in range(0, D, db):
                stage[d0 * 4:(d0 + db) * 4, :] = _pk(land[w, d0:d0 + db].reshape(db * HG, E))
            for p in range(HG // 2):
                for d0 in range(0, D, 128):
                    u = stage[pl.ds(d0 * 4 + p, 128, stride=4), :]
                    lo = pltpu.bitcast(u << 16, f32).astype(bf16)
                    hi = pltpu.bitcast(u & jnp.uint32(0xFFFF0000), f32).astype(bf16)
                    c_lo = pl.multiple_of(col0 + (2 * p) * E, E)
                    c_hi = pl.multiple_of(col0 + (2 * p + 1) * E, E)
                    dst[d0 // 2:d0 // 2 + 64, pl.ds(c_lo, E)] = _pk(lo)
                    dst[d0 // 2:d0 // 2 + 64, pl.ds(c_hi, E)] = _pk(hi)

        def proj_extra(w, col0):
            nb = 512
            for mb in range(NSEG * NX // 256):
                a = _upk(xe_p[mb * 128:(mb + 1) * 128, :])
                for nc in range(HG * E // nb):
                    c = pl.multiple_of(col0 + nc * nb, nb)
                    r = _dot(a, _upk(w_p[w][:, pl.ds(c, nb)]))
                    qkvx_s.at[:, w * HE:(w + 1) * HE][mb * 256:(mb + 1) * 256, pl.ds(c, nb)] = (
                        r.astype(bf16))


        def cp_xf():
            return pltpu.make_async_copy(x_hbm.at[:, 0:NF, :], x_s.at[:, 0:NF, :], sems.at[S_XF])

        cp_xe().start()
        for w in range(3):
            cp_chunk(w, 0).start()
        cp_mem().start()
        cp_wo(0).start()

        cp_xe().wait()
        sb = 16
        for s0 in range(0, NSEG, sb):
            xe = x_s[s0:s0 + sb, NF:SEG, :].astype(f32).reshape(sb * NX, D)
            xe_p[s0 * NX // 2:(s0 + sb) * NX // 2, :] = _pk(_ln(xe).astype(bf16))
        cp_chunk(0, 0).wait()
        relayout(0, wq_p, 0)
        cp_chunk(0, 1).start()

        def chunk_body(c, carry):
            g = c // 3
            w = c - 3 * g
            col = g * CW

            @pl.when(w == 0)
            def _():
                cp_chunk(1, g).wait()
                relayout(1, wk_p, col)
                proj_extra(0, col)

                @pl.when(g < NG - 1)
                def _():
                    cp_chunk(1, g + 1).start()

                @pl.when(g == 1)
                def _():
                    cp_xf().start()

                @pl.when(g == NG - 1)
                def _():
                    for cp in cp_b_first() + cp_b_rest():
                        cp.start()

            @pl.when(w == 1)
            def _():
                cp_chunk(2, g).wait()
                relayout(2, wv_p, col)
                proj_extra(1, col)

                @pl.when(g < NG - 1)
                def _():
                    cp_chunk(2, g + 1).start()

            @pl.when(w == 2)
            def _():
                @pl.when(g < NG - 1)
                def _():
                    cp_chunk(0, g + 1).wait()

                cp_wo(g).wait()
                relayout(0, wq_p.at[:, CW:], col)
                for r in range(0, CW, 128):
                    wo_p[r // 2:(r + 128) // 2, pl.ds(pl.multiple_of(col, CW), D)] = (
                        _pk(wo_l[r:r + 128, :]))
                proj_extra(2, col)

                @pl.when(g < NG - 2)
                def _():
                    cp_chunk(0, g + 2).start()

                @pl.when(g < NG - 1)
                def _():
                    cp_wo(g + 1).start()

            return carry

        lax.fori_loop(0, 3 * NG, chunk_body, 0)
        cp_xf().wait()
        cp_mem().wait()
        for cp in cp_b_first():
            cp.wait()

        scale = E ** -0.5
        row = lax.broadcasted_iota(jnp.int32, (L, LP), 0)
        col = lax.broadcasted_iota(jnp.int32, (L, LP), 1)
        allowed = (row < M) | (row >= col)
        valid = col < L
        zpad = jnp.zeros((LP - L, E), bf16)
        DS, DP = 1, 4
        WO_SPLIT = 8
        hs = H // WO_SPLIT

        def ln_fresh(s):
            xf = _ln(x_s[s, 0:NF, :].astype(f32))
            xf = jnp.concatenate([jnp.zeros((M, D), f32), xf], axis=0)
            xn_p[...] = _pk(xf.astype(bf16))

        ln_fresh(0)

        def step(s, mem):
            e0 = pl.multiple_of(s * NX, NX)
            lhs = _upk(jnp.concatenate([mem, xn_p[M // 2:, :]], axis=0))
            ln_fresh(jnp.minimum(s + 1, NSEG - 1))
            qs, ks, vs, ps, outs, ys = {}, {}, {}, {}, {}, []

            def proj(h):
                qs[h] = _dot(lhs, _upk(wq_p[:, h * E:(h + 1) * E]))
                ks[h] = _dot(lhs, _upk(wk_p[:, h * E:(h + 1) * E]))
                vs[h] = _dot(lhs, _upk(wv_p[:, h * E:(h + 1) * E]))

            def scores(h):
                qx = qkvx_s[pl.ds(e0, NX), h * E:(h + 1) * E]
                kx = qkvx_s[pl.ds(e0, NX), HE + h * E:HE + (h + 1) * E]
                q = jnp.concatenate([qs[h].astype(bf16), qx], axis=0)
                k = jnp.concatenate([ks[h].astype(bf16), kx, zpad], axis=0)
                sc = lax.dot_general(q, k, (((1,), (1,)), ((), ())),
                                     preferred_element_type=f32) * scale
                sc = jnp.where(allowed, sc, -1e9)
                sc = jnp.where(valid, sc, -jnp.inf)
                m = jnp.max(sc, axis=-1, keepdims=True)
                p = jnp.exp(sc - m)
                l = jnp.sum(p, axis=-1, keepdims=True)
                r = pl.reciprocal(l, approx=True)
                r = r * (2.0 - l * r)
                ps[h] = (p * r).astype(bf16)

            def pv(h):
                vx = qkvx_s[pl.ds(e0, NX), 2 * HE + h * E:2 * HE + (h + 1) * E]
                v = jnp.concatenate([vs[h].astype(bf16), vx, zpad], axis=0)
                o = _dot(ps[h], v)
                oex_s[pl.ds(e0, NX), h * E:(h + 1) * E] = o[NR:L].astype(bf16)
                outs[h] = o[0:NR].astype(bf16)

            def wo(j):
                oj = jnp.concatenate([outs[h] for h in range(j * hs, (j + 1) * hs)], axis=1)
                g, r = divmod(j * hs * E, CW)
                ys.append(_dot(oj, _upk(wo_p[r // 2:(r + hs * E) // 2, g * D:(g + 1) * D])))

            for t in range(H):
                proj(t)
                if t >= DS:
                    scores(t - DS)
                if t >= DP:
                    pv(t - DP)
            wo(0)
            wo(1)
            scores(H - 1)
            wo(2)
            wo(3)
            pv(H - 4)
            pv(H - 3)
            pv(H - 2)
            wo(4)
            wo(5)
            pv(H - 1)
            wo(6)
            wo(7)
            y = ys[0]
            for yy in ys[1:]:
                y = y + yy
            h_s[s, 0:NF, :] = x_s[s, 0:NF, :].astype(f32) + y[M:]
            return _pk(y[:M].astype(bf16))

        XG = NR // NX
        HALF = D // 2

        def wo_extra(grp, c0, n):
            e0 = pl.multiple_of(grp * NR, NR)
            s0 = pl.multiple_of(grp * XG, XG)
            y = None
            for g in range(NG):
                c = pl.multiple_of(g * D + c0, 128)
                yg = _dot(oex_s[pl.ds(e0, NR), g * CW:(g + 1) * CW], _upk(wo_p[:, pl.ds(c, n)]))
                y = yg if y is None else y + yg
            xe = x_s[pl.ds(s0, XG), NF:SEG, pl.ds(c0, n)].astype(f32)
            h_s[pl.ds(s0, XG), NF:SEG, pl.ds(c0, n)] = xe + y.reshape(XG, NX, n)

        oex_s[0:NR, :] = jnp.zeros((NR, HE), bf16)

        def pair(i, mem):
            @pl.when(i == 1)
            def _():
                for cp in cp_b_rest():
                    cp.wait()

            mem = step(2 * i, mem)
            wo_extra(jnp.maximum(i // 2 - 1, 0), pl.multiple_of((i % 2) * HALF, HALF), HALF)
            mem = step(2 * i + 1, mem)
            for src, dst, n in zip(b_land, b_pack, b_rows):
                dst[pl.ds(pl.multiple_of(i * (n // 2), n // 2), n // 2), :] = (
                    _pk(src[pl.ds(pl.multiple_of(i * n, n), n), :]))
            return mem

        lax.fori_loop(0, NPAIR, pair, _pk(mem0_s[...]))
        wo_extra(NSEG // XG - 1, 0, D)

    pl.run_scoped(
        phase_a,
        pltpu.VMEM((D // 2, HE + HG * E), u32),
        pltpu.VMEM((D // 2, HE), u32),
        pltpu.VMEM((D // 2, HE), u32),
        pltpu.VMEM((HG * E, D), bf16),
        pltpu.VMEM((HG * E // 2, NG * D), u32),
        pltpu.VMEM((3, D, HG, E), bf16),
        pltpu.VMEM((D * HG // 2, E), u32),
        pltpu.VMEM((NSEG * NX // 2, D), u32),
        pltpu.VMEM(((M + SEG - NX) // 2, D), u32),
        pltpu.VMEM((NSEG * NX, 3 * HE), bf16),
        pltpu.VMEM((NSEG * NX, HE), bf16),
    )

    NB = S // RB
    bseg = RB // SEG
    cq = D // 4

    def phase_b(g_s, a1_s, a_s, r_s, u_s, o_st):
        g_s[0:8, :] = jnp.zeros((8, D), f32)
        g_s[S + 8:S + 16, :] = jnp.zeros((8, D), f32)

        def load_h(i):
            return h_s[pl.ds(pl.multiple_of(i * bseg, bseg), bseg)].reshape(RB, D)

        def prep(i):
            return _pk(_ln2(load_h(i)).astype(bf16))

        def w1_stage(i):
            a = _upk(a1_s[...])
            r0 = pl.multiple_of(i * RB + 8, 8)
            for c in range(4):
                g = _gelu(_dot(a, _upk(w1_p[:, c * cq:(c + 1) * cq])))
                g_s[pl.ds(r0, RB), c * cq:(c + 1) * cq] = g

        def mix(i):
            r0 = pl.multiple_of(i * RB, RB)
            g0 = g_s[pl.ds(r0, RB + 16), 0 * cq:1 * cq][7:7 + RB]
            g1 = g_s[pl.ds(r0, RB + 16), 1 * cq:2 * cq][9:9 + RB]
            g2 = g_s[pl.ds(r0, RB + 16), 2 * cq:3 * cq][6:6 + RB]
            g3 = g_s[pl.ds(r0, RB + 16), 3 * cq:4 * cq][10:10 + RB]
            gs = jnp.concatenate([g0, g1, g2, g3], axis=1).astype(bf16)
            hsft = _dot(gs, _upk(w2_p[...]))
            hb = load_h(i)
            x1 = _ln(hb) + hsft
            a_s[...] = _pk(_ln(x1).astype(bf16))
            r_s[i % 2] = hb + x1

        def cp_out(i, slot):
            r0 = pl.multiple_of(i * RB, RB)
            return pltpu.make_async_copy(o_st.at[slot], out_hbm.at[pl.ds(r0, RB), :],
                                         sems.at[S_OUT + slot])

        def block(i, slot, with_prep, with_w1, with_mix):
            if with_w1:
                w1_stage(i + 2)
            if with_prep:
                a1_s[...] = prep(i + 3)
            a = _upk(a_s[...])
            for c in range(F // FC):
                u = _dot(a, _upk(w3_p[:, c * FC:(c + 1) * FC]))
                u_s[:, c * FC:(c + 1) * FC] = _pk(_gelu(u).astype(bf16))
            if with_mix:
                mix(i + 1)
            y = _dot(_upk(u_s[...]), _upk(w4_p[...]))
            o_st[slot] = (r_s[slot] + y).astype(bf16)
            cp_out(i, slot).start()

        a1_s[...] = prep(0)
        w1_stage(0)
        a1_s[...] = prep(1)
        w1_stage(1)
        a1_s[...] = prep(2)
        mix(0)

        def body(i, carry, **kw):
            slot = i % 2

            @pl.when(i >= 2)
            def _():
                cp_out(i - 2, slot).wait()

            block(i, slot, **kw)
            return carry

        lax.fori_loop(0, NB - 3, functools.partial(body, with_prep=True, with_w1=True, with_mix=True), 0)
        for i in range(NB - 3, NB):
            cp_out(i - 2, i % 2).wait()
            block(i, i % 2, with_prep=False, with_w1=i + 2 < NB, with_mix=i + 1 < NB)
        cp_out(NB - 2, (NB - 2) % 2).wait()
        cp_out(NB - 1, (NB - 1) % 2).wait()

    pl.run_scoped(
        phase_b,
        pltpu.VMEM((S + 16, D), f32),
        pltpu.VMEM((RB // 2, D), u32),
        pltpu.VMEM((RB // 2, D), u32),
        pltpu.VMEM((2, RB, D), f32),
        pltpu.VMEM((RB // 2, F), u32),
        pltpu.VMEM((2, RB, D), bf16),
    )


@functools.partial(jax.jit, static_argnames=("A_seg_len",))
def pallas_sequential_preLN__memory_aug_recurrent_mem_tr__mixer_s_mlp__prompt_kernel(
    A_x: jax.Array,
    A_mem0: jax.Array,
    A_Wq: jax.Array,
    A_Wk: jax.Array,
    A_Wv: jax.Array,
    A_Wo: jax.Array,
    A_seg_len: int,
    B_x: jax.Array,
    B_w1: jax.Array,
    B_w2: jax.Array,
    B_w3: jax.Array,
    B_w4: jax.Array,
):
    del B_x
    B, S, D = A_x.shape
    _, H, E = A_Wq.shape
    M = A_mem0.shape[1]
    F = B_w3.shape[1]
    SEG = int(A_seg_len)
    NSEG = S // SEG
    assert B == 1 and M == 8 and SEG == 32 and E == 128 and S == NSEG * SEG
    assert D == HG * E and H % HG == 0 and S % RB == 0 and F % FC == 0 and D % 256 == 0
    assert (NSEG * NX) % 256 == 0 and NSEG % (4 * (H // HG)) == 0 and NSEG % 16 == 0

    hbm = pl.BlockSpec(memory_space=pl.ANY)
    kernel = functools.partial(_kernel, NSEG=NSEG, SEG=SEG, D=D, H=H, E=E, M=M, F=F)
    out = pl.pallas_call(
        kernel,
        out_shape=jax.ShapeDtypeStruct((S, D), A_x.dtype),
        in_specs=[hbm] * 10,
        out_specs=hbm,
        scratch_shapes=[
            pltpu.VMEM((NSEG, SEG, D), bf16),
            pltpu.VMEM((NSEG, SEG, D), f32),
            pltpu.VMEM((M, D), bf16),
            pltpu.VMEM((D, D), bf16),
            pltpu.VMEM((D, D), bf16),
            pltpu.VMEM((D, F), bf16),
            pltpu.VMEM((F, D), bf16),
            pltpu.VMEM((D // 2, D), u32),
            pltpu.VMEM((D // 2, D), u32),
            pltpu.VMEM((D // 2, F), u32),
            pltpu.VMEM((F // 2, D), u32),
            pltpu.SemaphoreType.DMA((N_SEMS,)),
        ],
        compiler_params=pltpu.CompilerParams(vmem_limit_bytes=124 * 1024 * 1024),
        name="rmt_mixer",
    )(
        A_x.reshape(NSEG, SEG, D),
        A_mem0.reshape(M, D),
        A_Wq, A_Wk, A_Wv,
        A_Wo.reshape(H * E, D),
        B_w1, B_w2, B_w3, B_w4,
    )
    return out.reshape(B, S, D)
```

```python
import functools

import jax
import jax.numpy as jnp
from jax import lax
from jax.experimental import pallas as pl
from jax.experimental.pallas import tpu as pltpu

bf16, f32, u32 = jnp.bfloat16, jnp.float32, jnp.uint32

LN_EPS = 1e-5
NX = 8
HG = 8
RB = 128
FC = 512

S_XE, S_XF, S_LAND, S_WO, S_MEM, S_B0, S_B1, S_OUT = 0, 1, 2, 5, 6, 7, 11, 15
N_SEMS = 17


def _pk(x):
    return pltpu.bitcast(x, u32)


def _upk(x):
    return pltpu.bitcast(x, bf16)


def _dot(a, b):
    return jnp.dot(a, b, preferred_element_type=f32)


def _ln(x):
    m = jnp.mean(x, axis=-1, keepdims=True)
    xc = x - m
    v = jnp.mean(xc * xc, axis=-1, keepdims=True)
    return xc * lax.rsqrt(v + LN_EPS)


def _ln2(x):
    m = jnp.mean(x, axis=-1, keepdims=True)
    xc = x - m
    v = jnp.mean(xc * xc, axis=-1, keepdims=True)
    r = lax.rsqrt(v + LN_EPS)
    return xc * (r * lax.rsqrt(v * (r * r) + LN_EPS))


def _gelu(x):
    return 0.5 * x * (1.0 + jnp.tanh(0.7978845608028654 * (x + 0.044715 * (x * x * x))))


def _repack(src, dst, rows, blk):
    for r in range(0, rows, blk):
        dst[r // 2:(r + blk) // 2, :] = _pk(src[r:r + blk, :])


def _kernel(x_hbm, mem0_hbm, wq_hbm, wk_hbm, wv_hbm, wo_hbm, w1_hbm, w2_hbm, w3_hbm, w4_hbm,
            out_hbm,
            x_s, h_s, mem0_s, w1_l, w2_l, w3_l, w4_l, w1_p, w2_p, w3_p, w4_p, sems,
            *, NSEG, SEG, D, H, E, M, F):
    S = NSEG * SEG
    NF = SEG - NX
    NR = M + NF
    L = M + SEG
    LP = L + 8
    HE = H * E
    NG = H // HG
    w_hbm = (wq_hbm, wk_hbm, wv_hbm)

    def cp_xe():
        return pltpu.make_async_copy(x_hbm.at[:, NF:SEG, :], x_s.at[:, NF:SEG, :], sems.at[S_XE])

    XG = (M + SEG - NX) // NX
    NIT = NSEG // XG
    b_hbm = (w1_hbm, w2_hbm, w3_hbm, w4_hbm)
    b_land = (w1_l, w2_l, w3_l, w4_l)
    b_pack = (w1_p, w2_p, w3_p, w4_p)
    b_rows = tuple(r.shape[0] // NIT for r in b_hbm)

    def cp_b_first():
        return [pltpu.make_async_copy(h.at[0:n], l.at[0:n], sems.at[S_B0 + j])
                for j, (h, l, n) in enumerate(zip(b_hbm, b_land, b_rows))]

    def cp_b_rest():
        return [pltpu.make_async_copy(h.at[n:], l.at[n:], sems.at[S_B1 + j])
                for j, (h, l, n) in enumerate(zip(b_hbm, b_land, b_rows))]

    def cp_mem():
        return pltpu.make_async_copy(mem0_hbm, mem0_s, sems.at[S_MEM])

    def phase_a(wq_p, wk_p, wv_p, wo_l, wo_p, land, stage, xe_p, xn_p, qkvx_s, oex_s):
        w_p = (wq_p, wk_p, wv_p)
        CW = HG * E

        def cp_chunk(w, g):
            g0 = pl.multiple_of(g * HG, HG)
            return pltpu.make_async_copy(w_hbm[w].at[:, pl.ds(g0, HG), :], land.at[w],
                                         sems.at[S_LAND + w])

        def cp_wo(g):
            r0 = pl.multiple_of(g * CW, CW)
            return pltpu.make_async_copy(wo_hbm.at[pl.ds(r0, CW), :], wo_l, sems.at[S_WO])

        def relayout(w, dst, col0):
            db = 64
            for d0 in range(0, D, db):
                stage[d0 * 4:(d0 + db) * 4, :] = _pk(land[w, d0:d0 + db].reshape(db * HG, E))
            for p in range(HG // 2):
                for d0 in range(0, D, 128):
                    u = stage[pl.ds(d0 * 4 + p, 128, stride=4), :]
                    lo = pltpu.bitcast(u << 16, f32).astype(bf16)
                    hi = pltpu.bitcast(u & jnp.uint32(0xFFFF0000), f32).astype(bf16)
                    c_lo = pl.multiple_of(col0 + (2 * p) * E, E)
                    c_hi = pl.multiple_of(col0 + (2 * p + 1) * E, E)
                    dst[d0 // 2:d0 // 2 + 64, pl.ds(c_lo, E)] = _pk(lo)
                    dst[d0 // 2:d0 // 2 + 64, pl.ds(c_hi, E)] = _pk(hi)

        def proj_extra(w, col0):
            nb = 512
            for mb in range(NSEG * NX // 256):
                a = _upk(xe_p[mb * 128:(mb + 1) * 128, :])
                for nc in range(HG * E // nb):
                    c = pl.multiple_of(col0 + nc * nb, nb)
                    r = _dot(a, _upk(w_p[w][:, pl.ds(c, nb)]))
                    qkvx_s.at[:, w * HE:(w + 1) * HE][mb * 256:(mb + 1) * 256, pl.ds(c, nb)] = (
                        r.astype(bf16))


        def cp_xf():
            return pltpu.make_async_copy(x_hbm.at[:, 0:NF, :], x_s.at[:, 0:NF, :], sems.at[S_XF])

        cp_xe().start()
        for w in range(3):
            cp_chunk(w, 0).start()
        cp_mem().start()
        cp_wo(0).start()

        cp_xe().wait()
        sb = 16
        for s0 in range(0, NSEG, sb):
            xe = x_s[s0:s0 + sb, NF:SEG, :].astype(f32).reshape(sb * NX, D)
            xe_p[s0 * NX // 2:(s0 + sb) * NX // 2, :] = _pk(_ln(xe).astype(bf16))
        cp_chunk(0, 0).wait()
        relayout(0, wq_p, 0)
        cp_chunk(0, 1).start()
        proj_extra(0, 0)
        cp_chunk(1, 0).wait()
        relayout(1, wk_p, 0)
        cp_chunk(1, 1).start()

        def chunk_body(c, carry):
            g = c // 3
            w = c - 3 * g
            col = g * CW

            @pl.when(w == 0)
            def _():
                cp_chunk(1, g).wait()
                relayout(1, wk_p, col)
                proj_extra(0, col)

                @pl.when(g < NG - 1)
                def _():
                    cp_chunk(1, g + 1).start()

                @pl.when(g == 1)
                def _():
                    cp_xf().start()

                @pl.when(g == NG - 1)
                def _():
                    for cp in cp_b_first() + cp_b_rest():
                        cp.start()

            @pl.when(w == 1)
            def _():
                cp_chunk(2, g).wait()
                relayout(2, wv_p, col)
                proj_extra(1, col)

                @pl.when(g < NG - 1)
                def _():
                    cp_chunk(2, g + 1).start()

            @pl.when(w == 2)
            def _():
                @pl.when(g < NG - 1)
                def _():
                    cp_chunk(0, g + 1).wait()

                cp_wo(g).wait()
                relayout(0, wq_p.at[:, CW:], col)
                for r in range(0, CW, 128):
                    wo_p[r // 2:(r + 128) // 2, pl.ds(pl.multiple_of(col, CW), D)] = (
                        _pk(wo_l[r:r + 128, :]))
                proj_extra(2, col)

                @pl.when(g < NG - 2)
                def _():
                    cp_chunk(0, g + 2).start()

                @pl.when(g < NG - 1)
                def _():
                    cp_wo(g + 1).start()

            return carry

        lax.fori_loop(1, 3 * NG, chunk_body, 0)
        cp_xf().wait()
        cp_mem().wait()
        for cp in cp_b_first():
            cp.wait()

        scale = E ** -0.5
        zpad = jnp.zeros((LP - L, E), bf16)

        def masks(paired):
            shape = (NR + 2 * NX, 2 * L) if paired else (NR, LP)
            row = lax.broadcasted_iota(jnp.int32, shape, 0)
            col = lax.broadcasted_iota(jnp.int32, shape, 1)
            if not paired:
                return (row < M) | (row >= col), col < L
            prev_q = (row >= NR) & (row < L)
            prev_k = (col >= NR) & (col < NR + L)
            qi = jnp.where(row >= L, row - NX, row)
            kj = jnp.where(col < NR, col, jnp.where(prev_k, col - NR, col - L))
            return (qi < M) | (qi >= kj), prev_q == prev_k

        mask_tab = (masks(False), masks(True))
        DS, DP = 1, 4
        WO_SPLIT = 8
        hs = H // WO_SPLIT

        def ln_fresh(s):
            xf = _ln(x_s[s, 0:NF, :].astype(f32))
            xf = jnp.concatenate([jnp.zeros((M, D), f32), xf], axis=0)
            xn_p[...] = _pk(xf.astype(bf16))

        ln_fresh(0)

        def step(s, mem, prev):
            paired = prev is not None
            allowed, valid = mask_tab[paired]
            kvs = {}
            e0 = pl.multiple_of(s * NX, NX)
            ep = pl.multiple_of(s * NX - NX, 2 * NX) if paired else None
            lhs = _upk(jnp.concatenate([mem, xn_p[M // 2:, :]], axis=0))
            ln_fresh(jnp.minimum(s + 1, NSEG - 1))
            qs, ks, vs, ps, outs, ys = {}, {}, {}, {}, {}, []

            def proj(h):
                qs[h] = _dot(lhs, _upk(wq_p[:, h * E:(h + 1) * E]))
                ks[h] = _dot(lhs, _upk(wk_p[:, h * E:(h + 1) * E]))
                vs[h] = _dot(lhs, _upk(wv_p[:, h * E:(h + 1) * E]))

            def with_extra(cur, j, h, part):
                c0 = part * HE + h * E
                kvs.setdefault(h, {})[j] = cur
                if paired:
                    return jnp.concatenate(
                        [cur, prev[h][j], qkvx_s[pl.ds(ep, 2 * NX), c0:c0 + E]], axis=0)
                return jnp.concatenate([cur, qkvx_s[pl.ds(e0, NX), c0:c0 + E], zpad], axis=0)

            def scores(h):
                k = with_extra(ks[h].astype(bf16), 0, h, 1)
                q = qs[h].astype(bf16)
                if paired:
                    q = jnp.concatenate([q, qkvx_s[pl.ds(ep, 2 * NX), h * E:(h + 1) * E]], axis=0)
                sc = lax.dot_general(q, k, (((1,), (1,)), ((), ())),
                                     preferred_element_type=f32) * scale
                sc = jnp.where(allowed, sc, -1e9)
                sc = jnp.where(valid, sc, -jnp.inf)
                m = jnp.max(sc, axis=-1, keepdims=True)
                p = jnp.exp(sc - m)
                l = jnp.sum(p, axis=-1, keepdims=True)
                r = pl.reciprocal(l, approx=True)
                r = r * (2.0 - l * r)
                ps[h] = (p * r).astype(bf16)

            def pv(h):
                o = _dot(ps[h], with_extra(vs[h].astype(bf16), 1, h, 2))
                if paired:
                    oex_s[pl.ds(ep, 2 * NX), h * E:(h + 1) * E] = o[NR:].astype(bf16)
                outs[h] = o[0:NR].astype(bf16)

            def wo(j):
                oj = jnp.concatenate([outs[h] for h in range(j * hs, (j + 1) * hs)], axis=1)
                g, r = divmod(j * hs * E, CW)
                ys.append(_dot(oj, _upk(wo_p[r // 2:(r + hs * E) // 2, g * D:(g + 1) * D])))

            for t in range(H):
                proj(t)
                if t >= DS:
                    scores(t - DS)
                if t >= DP:
                    pv(t - DP)
            wo(0)
            wo(1)
            scores(H - 1)
            wo(2)
            wo(3)
            pv(H - 4)
            pv(H - 3)
            pv(H - 2)
            wo(4)
            wo(5)
            pv(H - 1)
            wo(6)
            wo(7)
            y = ys[0]
            for yy in ys[1:]:
                y = y + yy
            h_s[s, 0:NF, :] = x_s[s, 0:NF, :].astype(f32) + y[M:]
            return _pk(y[:M].astype(bf16)), kvs

        def wo_extra(grp, c0, n):
            e0 = pl.multiple_of(grp * NR, NR)
            s0 = pl.multiple_of(grp * XG, XG)
            y = None
            for g in range(NG):
                yg = _dot(oex_s[pl.ds(e0, NR), g * CW:(g + 1) * CW],
                          _upk(wo_p[:, g * D + c0:g * D + c0 + n]))
                y = yg if y is None else y + yg
            xe = x_s[pl.ds(s0, XG), NF:SEG, c0:c0 + n].astype(f32)
            h_s[pl.ds(s0, XG), NF:SEG, c0:c0 + n] = xe + y.reshape(XG, NX, n)

        oex_s[0:NR, :] = jnp.zeros((NR, HE), bf16)
        fill = (3 * D // 8, D // 4, 3 * D // 8)

        def steps(i, mem):
            @pl.when(i == 1)
            def _():
                for cp in cp_b_rest():
                    cp.wait()

            grp = jnp.maximum(i - 1, 0)
            c0 = 0
            kvs = None
            for j in range(XG):
                mem, kvs = step(XG * i + j, mem, kvs if j % 2 else None)
                if j < XG - 1:
                    wo_extra(grp, c0, fill[j])
                    c0 += fill[j]
            for src, dst, n in zip(b_land, b_pack, b_rows):
                dst[pl.ds(pl.multiple_of(i * (n // 2), n // 2), n // 2), :] = (
                    _pk(src[pl.ds(pl.multiple_of(i * n, n), n), :]))
            return mem

        lax.fori_loop(0, NIT, steps, _pk(mem0_s[...]))
        wo_extra(NIT - 1, 0, D)

    pl.run_scoped(
        phase_a,
        pltpu.VMEM((D // 2, HE + HG * E), u32),
        pltpu.VMEM((D // 2, HE), u32),
        pltpu.VMEM((D // 2, HE), u32),
        pltpu.VMEM((HG * E, D), bf16),
        pltpu.VMEM((HG * E // 2, NG * D), u32),
        pltpu.VMEM((3, D, HG, E), bf16),
        pltpu.VMEM((D * HG // 2, E), u32),
        pltpu.VMEM((NSEG * NX // 2, D), u32),
        pltpu.VMEM(((M + SEG - NX) // 2, D), u32),
        pltpu.VMEM((NSEG * NX, 3 * HE), bf16),
        pltpu.VMEM((NSEG * NX, HE), bf16),
    )

    NB = S // RB
    bseg = RB // SEG
    cq = D // 4

    def phase_b(g_s, a1_s, a_s, r_s, u_s, o_st):
        g_s[0:8, :] = jnp.zeros((8, D), f32)
        g_s[S + 8:S + 16, :] = jnp.zeros((8, D), f32)

        def load_h(i):
            return h_s[pl.ds(pl.multiple_of(i * bseg, bseg), bseg)].reshape(RB, D)

        def prep(i):
            return _pk(_ln2(load_h(i)).astype(bf16))

        def w1_stage(i):
            a = _upk(a1_s[...])
            r0 = pl.multiple_of(i * RB + 8, 8)
            for c in range(4):
                g = _gelu(_dot(a, _upk(w1_p[:, c * cq:(c + 1) * cq])))
                g_s[pl.ds(r0, RB), c * cq:(c + 1) * cq] = g

        def mix(i):
            r0 = pl.multiple_of(i * RB, RB)
            g0 = g_s[pl.ds(r0, RB + 16), 0 * cq:1 * cq][7:7 + RB]
            g1 = g_s[pl.ds(r0, RB + 16), 1 * cq:2 * cq][9:9 + RB]
            g2 = g_s[pl.ds(r0, RB + 16), 2 * cq:3 * cq][6:6 + RB]
            g3 = g_s[pl.ds(r0, RB + 16), 3 * cq:4 * cq][10:10 + RB]
            gs = jnp.concatenate([g0, g1, g2, g3], axis=1).astype(bf16)
            hsft = _dot(gs, _upk(w2_p[...]))
            hb = load_h(i)
            x1 = _ln(hb) + hsft
            a_s[...] = _pk(_ln(x1).astype(bf16))
            r_s[i % 2] = hb + x1

        def cp_out(i, slot):
            r0 = pl.multiple_of(i * RB, RB)
            return pltpu.make_async_copy(o_st.at[slot], out_hbm.at[pl.ds(r0, RB), :],
                                         sems.at[S_OUT + slot])

        def block(i, slot, with_prep, with_w1, with_mix):
            if with_w1:
                w1_stage(i + 2)
            if with_prep:
                a1_s[...] = prep(i + 3)
            a = _upk(a_s[...])
            for c in range(F // FC):
                u = _dot(a, _upk(w3_p[:, c * FC:(c + 1) * FC]))
                u_s[:, c * FC:(c + 1) * FC] = _pk(_gelu(u).astype(bf16))
            if with_mix:
                mix(i + 1)
            y = _dot(_upk(u_s[...]), _upk(w4_p[...]))
            o_st[slot] = (r_s[slot] + y).astype(bf16)
            cp_out(i, slot).start()

        a1_s[...] = prep(0)
        w1_stage(0)
        a1_s[...] = prep(1)
        w1_stage(1)
        a1_s[...] = prep(2)
        mix(0)

        def body(i, carry, **kw):
            slot = i % 2

            @pl.when(i >= 2)
            def _():
                cp_out(i - 2, slot).wait()

            block(i, slot, **kw)
            return carry

        lax.fori_loop(0, NB - 3, functools.partial(body, with_prep=True, with_w1=True, with_mix=True), 0)
        for i in range(NB - 3, NB):
            cp_out(i - 2, i % 2).wait()
            block(i, i % 2, with_prep=False, with_w1=i + 2 < NB, with_mix=i + 1 < NB)
        cp_out(NB - 2, (NB - 2) % 2).wait()
        cp_out(NB - 1, (NB - 1) % 2).wait()

    pl.run_scoped(
        phase_b,
        pltpu.VMEM((S + 16, D), f32),
        pltpu.VMEM((RB // 2, D), u32),
        pltpu.VMEM((RB // 2, D), u32),
        pltpu.VMEM((2, RB, D), f32),
        pltpu.VMEM((RB // 2, F), u32),
        pltpu.VMEM((2, RB, D), bf16),
    )


@functools.partial(jax.jit, static_argnames=("A_seg_len",))
def pallas_sequential_preLN__memory_aug_recurrent_mem_tr__mixer_s_mlp__prompt_kernel(
    A_x: jax.Array,
    A_mem0: jax.Array,
    A_Wq: jax.Array,
    A_Wk: jax.Array,
    A_Wv: jax.Array,
    A_Wo: jax.Array,
    A_seg_len: int,
    B_x: jax.Array,
    B_w1: jax.Array,
    B_w2: jax.Array,
    B_w3: jax.Array,
    B_w4: jax.Array,
):
    del B_x
    B, S, D = A_x.shape
    _, H, E = A_Wq.shape
    M = A_mem0.shape[1]
    F = B_w3.shape[1]
    SEG = int(A_seg_len)
    NSEG = S // SEG
    assert B == 1 and M == 8 and SEG == 32 and E == 128 and S == NSEG * SEG
    assert D == HG * E and H % HG == 0 and S % RB == 0 and F % FC == 0 and D % 256 == 0
    assert (NSEG * NX) % 256 == 0 and NSEG % (4 * (H // HG)) == 0 and NSEG % 16 == 0

    hbm = pl.BlockSpec(memory_space=pl.ANY)
    kernel = functools.partial(_kernel, NSEG=NSEG, SEG=SEG, D=D, H=H, E=E, M=M, F=F)
    out = pl.pallas_call(
        kernel,
        out_shape=jax.ShapeDtypeStruct((S, D), A_x.dtype),
        in_specs=[hbm] * 10,
        out_specs=hbm,
        scratch_shapes=[
            pltpu.VMEM((NSEG, SEG, D), bf16),
            pltpu.VMEM((NSEG, SEG, D), f32),
            pltpu.VMEM((M, D), bf16),
            pltpu.VMEM((D, D), bf16),
            pltpu.VMEM((D, D), bf16),
            pltpu.VMEM((D, F), bf16),
            pltpu.VMEM((F, D), bf16),
            pltpu.VMEM((D // 2, D), u32),
            pltpu.VMEM((D // 2, D), u32),
            pltpu.VMEM((D // 2, F), u32),
            pltpu.VMEM((F // 2, D), u32),
            pltpu.SemaphoreType.DMA((N_SEMS,)),
        ],
        compiler_params=pltpu.CompilerParams(vmem_limit_bytes=124 * 1024 * 1024),
        name="rmt_mixer",
    )(
        A_x.reshape(NSEG, SEG, D),
        A_mem0.reshape(M, D),
        A_Wq, A_Wk, A_Wv,
        A_Wo.reshape(H * E, D),
        B_w1, B_w2, B_w3, B_w4,
    )
    return out.reshape(B, S, D)
```

```python
import functools

import jax
import jax.numpy as jnp
from jax import lax
from jax.experimental import pallas as pl
from jax.experimental.pallas import tpu as pltpu

bf16, f32, u32 = jnp.bfloat16, jnp.float32, jnp.uint32

LN_EPS = 1e-5
NX = 8
HG = 8
RB = 128
FC = 512

S_XE, S_XF, S_LAND, S_WO, S_MEM, S_B0, S_B1, S_OUT = 0, 1, 2, 5, 6, 7, 11, 15
N_SEMS = 17


def _pk(x):
    return pltpu.bitcast(x, u32)


def _upk(x):
    return pltpu.bitcast(x, bf16)


def _dot(a, b):
    return jnp.dot(a, b, preferred_element_type=f32)


def _ln(x):
    m = jnp.mean(x, axis=-1, keepdims=True)
    xc = x - m
    v = jnp.mean(xc * xc, axis=-1, keepdims=True)
    return xc * lax.rsqrt(v + LN_EPS)


def _ln2(x):
    m = jnp.mean(x, axis=-1, keepdims=True)
    xc = x - m
    v = jnp.mean(xc * xc, axis=-1, keepdims=True)
    r = lax.rsqrt(v + LN_EPS)
    return xc * (r * lax.rsqrt(v * (r * r) + LN_EPS))


def _gelu(x):
    c = 0.7978845608028654
    return x * (0.5 + 0.5 * jnp.tanh(x * (c + (c * 0.044715) * (x * x))))


def _repack(src, dst, rows, blk):
    for r in range(0, rows, blk):
        dst[r // 2:(r + blk) // 2, :] = _pk(src[r:r + blk, :])


def _kernel(x_hbm, mem0_hbm, wq_hbm, wk_hbm, wv_hbm, wo_hbm, w1_hbm, w2_hbm, w3_hbm, w4_hbm,
            out_hbm,
            x_s, h_s, mem0_s, w1_l, w2_l, w3_l, w4_l, w1_p, w2_p, w3_p, w4_p, sems,
            *, NSEG, SEG, D, H, E, M, F):
    S = NSEG * SEG
    NF = SEG - NX
    NR = M + NF
    L = M + SEG
    LP = L + 8
    HE = H * E
    NG = H // HG
    w_hbm = (wq_hbm, wk_hbm, wv_hbm)

    def cp_xe():
        return pltpu.make_async_copy(x_hbm.at[:, NF:SEG, :], x_s.at[:, NF:SEG, :], sems.at[S_XE])

    XG = (M + SEG - NX) // NX
    NIT = NSEG // 2
    b_hbm = (w1_hbm, w2_hbm, w3_hbm, w4_hbm)
    b_land = (w1_l, w2_l, w3_l, w4_l)
    b_pack = (w1_p, w2_p, w3_p, w4_p)
    b_rows = tuple(r.shape[0] // NIT for r in b_hbm)

    def cp_b_first():
        return [pltpu.make_async_copy(h.at[0:n], l.at[0:n], sems.at[S_B0 + j])
                for j, (h, l, n) in enumerate(zip(b_hbm, b_land, b_rows))]

    def cp_b_rest():
        return [pltpu.make_async_copy(h.at[n:], l.at[n:], sems.at[S_B1 + j])
                for j, (h, l, n) in enumerate(zip(b_hbm, b_land, b_rows))]

    def cp_mem():
        return pltpu.make_async_copy(mem0_hbm, mem0_s, sems.at[S_MEM])

    def phase_a(wq_p, wk_p, wv_p, wo_l, wo_p, land, stage, xe_p, xn_p, qkvx_s, oex_s):
        w_p = (wq_p, wk_p, wv_p)
        CW = HG * E

        def cp_chunk(w, g):
            g0 = pl.multiple_of(g * HG, HG)
            return pltpu.make_async_copy(w_hbm[w].at[:, pl.ds(g0, HG), :], land.at[w],
                                         sems.at[S_LAND + w])

        def cp_wo(g):
            r0 = pl.multiple_of(g * CW, CW)
            return pltpu.make_async_copy(wo_hbm.at[pl.ds(r0, CW), :], wo_l, sems.at[S_WO])

        def relayout(w, dst, col0):
            db = 64
            for d0 in range(0, D, db):
                stage[d0 * 4:(d0 + db) * 4, :] = _pk(land[w, d0:d0 + db].reshape(db * HG, E))
            for p in range(HG // 2):
                for d0 in range(0, D, 128):
                    u = stage[pl.ds(d0 * 4 + p, 128, stride=4), :]
                    lo = pltpu.bitcast(u << 16, f32).astype(bf16)
                    hi = pltpu.bitcast(u & jnp.uint32(0xFFFF0000), f32).astype(bf16)
                    c_lo = pl.multiple_of(col0 + (2 * p) * E, E)
                    c_hi = pl.multiple_of(col0 + (2 * p + 1) * E, E)
                    dst[d0 // 2:d0 // 2 + 64, pl.ds(c_lo, E)] = _pk(lo)
                    dst[d0 // 2:d0 // 2 + 64, pl.ds(c_hi, E)] = _pk(hi)

        def proj_extra(w, col0):
            nb = 512
            for mb in range(NSEG * NX // 256):
                a = _upk(xe_p[mb * 128:(mb + 1) * 128, :])
                for nc in range(HG * E // nb):
                    c = pl.multiple_of(col0 + nc * nb, nb)
                    r = _dot(a, _upk(w_p[w][:, pl.ds(c, nb)]))
                    qkvx_s.at[:, w * HE:(w + 1) * HE][mb * 256:(mb + 1) * 256, pl.ds(c, nb)] = (
                        r.astype(bf16))


        def cp_xf():
            return pltpu.make_async_copy(x_hbm.at[:, 0:NF, :], x_s.at[:, 0:NF, :], sems.at[S_XF])

        cp_chunk(0, 0).start()
        cp_xe().start()
        cp_chunk(1, 0).start()
        cp_chunk(2, 0).start()
        cp_mem().start()
        cp_wo(0).start()

        cp_chunk(0, 0).wait()
        relayout(0, wq_p, 0)
        cp_chunk(0, 1).start()
        cp_xe().wait()
        sb = 16
        for s0 in range(0, NSEG, sb):
            xe = x_s[s0:s0 + sb, NF:SEG, :].astype(f32).reshape(sb * NX, D)
            xe_p[s0 * NX // 2:(s0 + sb) * NX // 2, :] = _pk(_ln(xe).astype(bf16))
        proj_extra(0, 0)
        cp_chunk(1, 0).wait()
        relayout(1, wk_p, 0)
        cp_chunk(1, 1).start()

        def chunk_body(c, carry):
            g = c // 3
            w = c - 3 * g
            col = g * CW

            @pl.when(w == 0)
            def _():
                cp_chunk(1, g).wait()
                relayout(1, wk_p, col)
                proj_extra(0, col)

                @pl.when(g < NG - 1)
                def _():
                    cp_chunk(1, g + 1).start()

                @pl.when(g == 1)
                def _():
                    cp_xf().start()

            @pl.when(w == 1)
            def _():
                cp_chunk(2, g).wait()
                relayout(2, wv_p, col)
                proj_extra(1, col)

                @pl.when(g < NG - 1)
                def _():
                    cp_chunk(2, g + 1).start()

            @pl.when(w == 2)
            def _():
                @pl.when(g < NG - 1)
                def _():
                    cp_chunk(0, g + 1).wait()

                cp_wo(g).wait()
                relayout(0, wq_p.at[:, CW:], col)
                for r in range(0, CW, 128):
                    wo_p[r // 2:(r + 128) // 2, pl.ds(pl.multiple_of(col, CW), D)] = (
                        _pk(wo_l[r:r + 128, :]))
                proj_extra(2, col)

                @pl.when(g < NG - 2)
                def _():
                    cp_chunk(0, g + 2).start()

                @pl.when(g < NG - 1)
                def _():
                    cp_wo(g + 1).start()

                @pl.when(g == NG - 2)
                def _():
                    for cp in cp_b_first() + cp_b_rest():
                        cp.start()

            return carry

        lax.fori_loop(1, 3 * NG, chunk_body, 0)
        cp_xf().wait()
        cp_mem().wait()
        for cp in cp_b_first():
            cp.wait()

        scale = E ** -0.5
        zpad = jnp.zeros((LP - L, E), bf16)

        def masks(paired):
            shape = (NR + 2 * NX, 2 * L) if paired else (NR, LP)
            row = lax.broadcasted_iota(jnp.int32, shape, 0)
            col = lax.broadcasted_iota(jnp.int32, shape, 1)
            if not paired:
                return (row < M) | (row >= col), col < L
            prev_q = (row >= NR) & (row < L)
            prev_k = (col >= NR) & (col < NR + L)
            qi = jnp.where(row >= L, row - NX, row)
            kj = jnp.where(col < NR, col, jnp.where(prev_k, col - NR, col - L))
            return (qi < M) | (qi >= kj), prev_q == prev_k

        mask_tab = (masks(False), masks(True))
        DS, DP = 1, 4
        WO_SPLIT = 8
        hs = H // WO_SPLIT

        def ln_fresh(s):
            xf = _ln(x_s[s, 0:NF, :].astype(f32))
            xf = jnp.concatenate([jnp.zeros((M, D), f32), xf], axis=0)
            xn_p[...] = _pk(xf.astype(bf16))

        ln_fresh(0)

        def step(s, mem, prev):
            paired = prev is not None
            allowed, valid = mask_tab[paired]
            kvs = {}
            e0 = pl.multiple_of(s * NX, NX)
            ep = pl.multiple_of(s * NX - NX, 2 * NX) if paired else None
            lhs = _upk(jnp.concatenate([mem, xn_p[M // 2:, :]], axis=0))
            ln_fresh(jnp.minimum(s + 1, NSEG - 1))
            qs, ks, vs, ps, outs, ys = {}, {}, {}, {}, {}, []

            def proj(h):
                qs[h] = _dot(lhs, _upk(wq_p[:, h * E:(h + 1) * E]))
                ks[h] = _dot(lhs, _upk(wk_p[:, h * E:(h + 1) * E]))
                vs[h] = _dot(lhs, _upk(wv_p[:, h * E:(h + 1) * E]))

            def with_extra(cur, j, h, part):
                c0 = part * HE + h * E
                kvs.setdefault(h, {})[j] = cur
                if paired:
                    return jnp.concatenate(
                        [cur, prev[h][j], qkvx_s[pl.ds(ep, 2 * NX), c0:c0 + E]], axis=0)
                return jnp.concatenate([cur, qkvx_s[pl.ds(e0, NX), c0:c0 + E], zpad], axis=0)

            def scores(h):
                k = with_extra(ks[h].astype(bf16), 0, h, 1)
                q = qs[h].astype(bf16)
                if paired:
                    q = jnp.concatenate([q, qkvx_s[pl.ds(ep, 2 * NX), h * E:(h + 1) * E]], axis=0)
                sc = lax.dot_general(q, k, (((1,), (1,)), ((), ())),
                                     preferred_element_type=f32) * scale
                sc = jnp.where(allowed, sc, -1e9)
                sc = jnp.where(valid, sc, -jnp.inf)
                m = jnp.max(sc, axis=-1, keepdims=True)
                p = jnp.exp(sc - m)
                l = jnp.sum(p, axis=-1, keepdims=True)
                r = pl.reciprocal(l, approx=True)
                r = r * (2.0 - l * r)
                ps[h] = (p * r).astype(bf16)

            def pv(h):
                o = _dot(ps[h], with_extra(vs[h].astype(bf16), 1, h, 2))
                if paired:
                    oex_s[pl.ds(ep, 2 * NX), h * E:(h + 1) * E] = o[NR:].astype(bf16)
                outs[h] = o[0:NR].astype(bf16)

            def wo(j):
                oj = jnp.concatenate([outs[h] for h in range(j * hs, (j + 1) * hs)], axis=1)
                g, r = divmod(j * hs * E, CW)
                ys.append(_dot(oj, _upk(wo_p[r // 2:(r + hs * E) // 2, g * D:(g + 1) * D])))

            for t in range(H):
                proj(t)
                if t >= DS:
                    scores(t - DS)
                if t >= DP:
                    pv(t - DP)
            wo(0)
            wo(1)
            scores(H - 1)
            wo(2)
            wo(3)
            pv(H - 4)
            pv(H - 3)
            pv(H - 2)
            wo(4)
            wo(5)
            pv(H - 1)
            wo(6)
            wo(7)
            y = ys[0]
            for yy in ys[1:]:
                y = y + yy
            h_s[s, 0:NF, :] = x_s[s, 0:NF, :].astype(f32) + y[M:]
            return _pk(y[:M].astype(bf16)), kvs

        def wo_extra(grp, c0, n):
            e0 = pl.multiple_of(grp * NR, NR)
            s0 = pl.multiple_of(grp * XG, XG)
            y = None
            for g in range(NG):
                c = pl.multiple_of(g * D + c0, 128)
                yg = _dot(oex_s[pl.ds(e0, NR), g * CW:(g + 1) * CW], _upk(wo_p[:, pl.ds(c, n)]))
                y = yg if y is None else y + yg
            xe = x_s[pl.ds(s0, XG), NF:SEG, pl.ds(c0, n)].astype(f32)
            h_s[pl.ds(s0, XG), NF:SEG, pl.ds(c0, n)] = xe + y.reshape(XG, NX, n)

        oex_s[0:NR, :] = jnp.zeros((NR, HE), bf16)
        HALF = D // 2

        def steps(i, mem):
            @pl.when(i == 1)
            def _():
                for cp in cp_b_rest():
                    cp.wait()

            mem, kvs = step(2 * i, mem, None)
            wo_extra(jnp.maximum(i // 2 - 1, 0), pl.multiple_of((i % 2) * HALF, HALF), HALF)
            mem, _ = step(2 * i + 1, mem, kvs)
            for src, dst, n in zip(b_land, b_pack, b_rows):
                dst[pl.ds(pl.multiple_of(i * (n // 2), n // 2), n // 2), :] = (
                    _pk(src[pl.ds(pl.multiple_of(i * n, n), n), :]))
            return mem

        lax.fori_loop(0, NIT, steps, _pk(mem0_s[...]))
        wo_extra(NSEG // XG - 1, 0, D)

    pl.run_scoped(
        phase_a,
        pltpu.VMEM((D // 2, HE + HG * E), u32),
        pltpu.VMEM((D // 2, HE), u32),
        pltpu.VMEM((D // 2, HE), u32),
        pltpu.VMEM((HG * E, D), bf16),
        pltpu.VMEM((HG * E // 2, NG * D), u32),
        pltpu.VMEM((3, D, HG, E), bf16),
        pltpu.VMEM((D * HG // 2, E), u32),
        pltpu.VMEM((NSEG * NX // 2, D), u32),
        pltpu.VMEM(((M + SEG - NX) // 2, D), u32),
        pltpu.VMEM((NSEG * NX, 3 * HE), bf16),
        pltpu.VMEM((NSEG * NX, HE), bf16),
    )

    NB = S // RB
    bseg = RB // SEG
    cq = D // 4

    def phase_b(g_s, a1_s, a_s, r_s, u_s, o_st):
        g_s[0:8, :] = jnp.zeros((8, D), f32)
        g_s[S + 8:S + 16, :] = jnp.zeros((8, D), f32)

        def load_h(i):
            return h_s[pl.ds(pl.multiple_of(i * bseg, bseg), bseg)].reshape(RB, D)

        def prep(i):
            return _pk(_ln2(load_h(i)).astype(bf16))

        def w1_stage(i):
            a = _upk(a1_s[...])
            r0 = pl.multiple_of(i * RB + 8, 8)
            for c in range(4):
                g = _gelu(_dot(a, _upk(w1_p[:, c * cq:(c + 1) * cq])))
                g_s[pl.ds(r0, RB), c * cq:(c + 1) * cq] = g

        def mix(i):
            r0 = pl.multiple_of(i * RB, RB)
            g0 = g_s[pl.ds(r0, RB + 16), 0 * cq:1 * cq][7:7 + RB]
            g1 = g_s[pl.ds(r0, RB + 16), 1 * cq:2 * cq][9:9 + RB]
            g2 = g_s[pl.ds(r0, RB + 16), 2 * cq:3 * cq][6:6 + RB]
            g3 = g_s[pl.ds(r0, RB + 16), 3 * cq:4 * cq][10:10 + RB]
            gs = jnp.concatenate([g0, g1, g2, g3], axis=1).astype(bf16)
            hsft = _dot(gs, _upk(w2_p[...]))
            hb = load_h(i)
            x1 = _ln(hb) + hsft
            a_s[...] = _pk(_ln(x1).astype(bf16))
            r_s[i % 2] = hb + x1

        def cp_out(i, slot):
            r0 = pl.multiple_of(i * RB, RB)
            return pltpu.make_async_copy(o_st.at[slot], out_hbm.at[pl.ds(r0, RB), :],
                                         sems.at[S_OUT + slot])

        def block(i, slot, with_prep, with_w1, with_mix):
            if with_w1:
                w1_stage(i + 2)
            if with_prep:
                a1_s[...] = prep(i + 3)
            a = _upk(a_s[...])
            for c in range(F // FC):
                u = _dot(a, _upk(w3_p[:, c * FC:(c + 1) * FC]))
                u_s[:, c * FC:(c + 1) * FC] = _pk(_gelu(u).astype(bf16))
            if with_mix:
                mix(i + 1)
            y = _dot(_upk(u_s[...]), _upk(w4_p[...]))
            o_st[slot] = (r_s[slot] + y).astype(bf16)
            cp_out(i, slot).start()

        a1_s[...] = prep(0)
        w1_stage(0)
        a1_s[...] = prep(1)
        w1_stage(1)
        a1_s[...] = prep(2)
        mix(0)

        def body(i, carry, **kw):
            slot = i % 2

            @pl.when(i >= 2)
            def _():
                cp_out(i - 2, slot).wait()

            block(i, slot, **kw)
            return carry

        lax.fori_loop(0, NB - 3, functools.partial(body, with_prep=True, with_w1=True, with_mix=True), 0)
        for i in range(NB - 3, NB):
            cp_out(i - 2, i % 2).wait()
            block(i, i % 2, with_prep=False, with_w1=i + 2 < NB, with_mix=i + 1 < NB)
        cp_out(NB - 2, (NB - 2) % 2).wait()
        cp_out(NB - 1, (NB - 1) % 2).wait()

    pl.run_scoped(
        phase_b,
        pltpu.VMEM((S + 16, D), f32),
        pltpu.VMEM((RB // 2, D), u32),
        pltpu.VMEM((RB // 2, D), u32),
        pltpu.VMEM((2, RB, D), f32),
        pltpu.VMEM((RB // 2, F), u32),
        pltpu.VMEM((2, RB, D), bf16),
    )


@functools.partial(jax.jit, static_argnames=("A_seg_len",))
def pallas_sequential_preLN__memory_aug_recurrent_mem_tr__mixer_s_mlp__prompt_kernel(
    A_x: jax.Array,
    A_mem0: jax.Array,
    A_Wq: jax.Array,
    A_Wk: jax.Array,
    A_Wv: jax.Array,
    A_Wo: jax.Array,
    A_seg_len: int,
    B_x: jax.Array,
    B_w1: jax.Array,
    B_w2: jax.Array,
    B_w3: jax.Array,
    B_w4: jax.Array,
):
    del B_x
    B, S, D = A_x.shape
    _, H, E = A_Wq.shape
    M = A_mem0.shape[1]
    F = B_w3.shape[1]
    SEG = int(A_seg_len)
    NSEG = S // SEG
    assert B == 1 and M == 8 and SEG == 32 and E == 128 and S == NSEG * SEG
    assert D == HG * E and H % HG == 0 and S % RB == 0 and F % FC == 0 and D % 256 == 0
    assert (NSEG * NX) % 256 == 0 and NSEG % (4 * (H // HG)) == 0 and NSEG % 16 == 0

    hbm = pl.BlockSpec(memory_space=pl.ANY)
    kernel = functools.partial(_kernel, NSEG=NSEG, SEG=SEG, D=D, H=H, E=E, M=M, F=F)
    out = pl.pallas_call(
        kernel,
        out_shape=jax.ShapeDtypeStruct((S, D), A_x.dtype),
        in_specs=[hbm] * 10,
        out_specs=hbm,
        scratch_shapes=[
            pltpu.VMEM((NSEG, SEG, D), bf16),
            pltpu.VMEM((NSEG, SEG, D), f32),
            pltpu.VMEM((M, D), bf16),
            pltpu.VMEM((D, D), bf16),
            pltpu.VMEM((D, D), bf16),
            pltpu.VMEM((D, F), bf16),
            pltpu.VMEM((F, D), bf16),
            pltpu.VMEM((D // 2, D), u32),
            pltpu.VMEM((D // 2, D), u32),
            pltpu.VMEM((D // 2, F), u32),
            pltpu.VMEM((F // 2, D), u32),
            pltpu.SemaphoreType.DMA((N_SEMS,)),
        ],
        compiler_params=pltpu.CompilerParams(vmem_limit_bytes=124 * 1024 * 1024),
        name="rmt_mixer",
    )(
        A_x.reshape(NSEG, SEG, D),
        A_mem0.reshape(M, D),
        A_Wq, A_Wk, A_Wv,
        A_Wo.reshape(H * E, D),
        B_w1, B_w2, B_w3, B_w4,
    )
    return out.reshape(B, S, D)
```

```python
import functools

import jax
import jax.numpy as jnp
from jax import lax
from jax.experimental import pallas as pl
from jax.experimental.pallas import tpu as pltpu

bf16, f32, u32 = jnp.bfloat16, jnp.float32, jnp.uint32

LN_EPS = 1e-5
NX = 8
HG = 8
RB = 128
FC = 512

S_XE, S_XF, S_LAND, S_WO, S_MEM, S_B0, S_B1, S_OUT = 0, 1, 2, 5, 6, 7, 11, 15
N_SEMS = 17


def _pk(x):
    return pltpu.bitcast(x, u32)


def _upk(x):
    return pltpu.bitcast(x, bf16)


def _dot(a, b):
    return jnp.dot(a, b, preferred_element_type=f32)


def _ln(x):
    m = jnp.mean(x, axis=-1, keepdims=True)
    xc = x - m
    v = jnp.mean(xc * xc, axis=-1, keepdims=True)
    return xc * lax.rsqrt(v + LN_EPS)


def _ln2(x):
    m = jnp.mean(x, axis=-1, keepdims=True)
    xc = x - m
    v = jnp.mean(xc * xc, axis=-1, keepdims=True)
    r = lax.rsqrt(v + LN_EPS)
    return xc * (r * lax.rsqrt(v * (r * r) + LN_EPS))


def _gelu(x):
    c = 0.7978845608028654
    return x * (0.5 + 0.5 * jnp.tanh(x * (c + (c * 0.044715) * (x * x))))


def _kernel(x_hbm, mem0_hbm, wq_hbm, wk_hbm, wv_hbm, wo_hbm, w1_hbm, w2_hbm, w3_hbm, w4_hbm,
            out_hbm,
            x_s, h_s, mem0_s, w1_l, w2_l, w3_l, w4_l, w1_p, w2_p, w3_p, w4_p, sems,
            *, NSEG, SEG, D, H, E, M, F):
    S = NSEG * SEG
    NF = SEG - NX
    NR = M + NF
    L = M + SEG
    LP = L + 8
    HE = H * E
    NG = H // HG
    w_hbm = (wq_hbm, wk_hbm, wv_hbm)

    def cp_xe():
        return pltpu.make_async_copy(x_hbm.at[:, NF:SEG, :], x_s.at[:, NF:SEG, :], sems.at[S_XE])

    XG = (M + SEG - NX) // NX
    NIT = NSEG // 2
    b_hbm = (w1_hbm, w2_hbm, w3_hbm, w4_hbm)
    b_land = (w1_l, w2_l, w3_l, w4_l)
    b_pack = (w1_p, w2_p, w3_p, w4_p)
    b_rows = tuple(r.shape[0] // NIT for r in b_hbm)

    def cp_b_first():
        return [pltpu.make_async_copy(h.at[0:n], l.at[0:n], sems.at[S_B0 + j])
                for j, (h, l, n) in enumerate(zip(b_hbm, b_land, b_rows))]

    def cp_b_rest():
        return [pltpu.make_async_copy(h.at[n:], l.at[n:], sems.at[S_B1 + j])
                for j, (h, l, n) in enumerate(zip(b_hbm, b_land, b_rows))]

    def cp_mem():
        return pltpu.make_async_copy(mem0_hbm, mem0_s, sems.at[S_MEM])

    def phase_a(wq_p, wk_p, wv_p, wo_l, wo_p, land, stage, xe_p, xn_p, qkvx_s, oex_s):
        w_p = (wq_p, wk_p, wv_p)
        CW = HG * E

        def cp_chunk(w, g):
            g0 = pl.multiple_of(g * HG, HG)
            return pltpu.make_async_copy(w_hbm[w].at[:, pl.ds(g0, HG), :], land.at[w],
                                         sems.at[S_LAND + w])

        def cp_wo(g):
            r0 = pl.multiple_of(g * CW, CW)
            return pltpu.make_async_copy(wo_hbm.at[pl.ds(r0, CW), :], wo_l, sems.at[S_WO])

        def relayout(w, dst, col0):
            db = 64
            for d0 in range(0, D, db):
                stage[d0 * 4:(d0 + db) * 4, :] = _pk(land[w, d0:d0 + db].reshape(db * HG, E))
            for p in range(HG // 2):
                for d0 in range(0, D, 128):
                    u = stage[pl.ds(d0 * 4 + p, 128, stride=4), :]
                    lo = pltpu.bitcast(u << 16, f32).astype(bf16)
                    hi = pltpu.bitcast(u & jnp.uint32(0xFFFF0000), f32).astype(bf16)
                    c_lo = pl.multiple_of(col0 + (2 * p) * E, E)
                    c_hi = pl.multiple_of(col0 + (2 * p + 1) * E, E)
                    dst[d0 // 2:d0 // 2 + 64, pl.ds(c_lo, E)] = _pk(lo)
                    dst[d0 // 2:d0 // 2 + 64, pl.ds(c_hi, E)] = _pk(hi)

        def proj_extra(w, col0):
            nb = 512
            for mb in range(NSEG * NX // 256):
                a = _upk(xe_p[mb * 128:(mb + 1) * 128, :])
                for nc in range(HG * E // nb):
                    c = pl.multiple_of(col0 + nc * nb, nb)
                    r = _dot(a, _upk(w_p[w][:, pl.ds(c, nb)]))
                    qkvx_s.at[:, w * HE:(w + 1) * HE][mb * 256:(mb + 1) * 256, pl.ds(c, nb)] = (
                        r.astype(bf16))

        def cp_xf():
            return pltpu.make_async_copy(x_hbm.at[:, 0:NF, :], x_s.at[:, 0:NF, :], sems.at[S_XF])

        cp_chunk(0, 0).start()
        cp_xe().start()
        cp_chunk(1, 0).start()
        cp_chunk(2, 0).start()
        cp_mem().start()
        cp_wo(0).start()

        cp_chunk(0, 0).wait()
        relayout(0, wq_p, 0)
        cp_chunk(0, 1).start()
        cp_xe().wait()
        sb = 16
        for s0 in range(0, NSEG, sb):
            xe = x_s[s0:s0 + sb, NF:SEG, :].astype(f32).reshape(sb * NX, D)
            xe_p[s0 * NX // 2:(s0 + sb) * NX // 2, :] = _pk(_ln(xe).astype(bf16))
        proj_extra(0, 0)
        cp_chunk(1, 0).wait()
        relayout(1, wk_p, 0)
        cp_chunk(1, 1).start()

        def chunk_body(c, carry):
            g = c // 3
            w = c - 3 * g
            col = g * CW

            @pl.when(w == 0)
            def _():
                cp_chunk(1, g).wait()
                relayout(1, wk_p, col)
                proj_extra(0, col)

                @pl.when(g < NG - 1)
                def _():
                    cp_chunk(1, g + 1).start()

                @pl.when(g == 1)
                def _():
                    cp_xf().start()

            @pl.when(w == 1)
            def _():
                cp_chunk(2, g).wait()
                relayout(2, wv_p, col)
                proj_extra(1, col)

                @pl.when(g < NG - 1)
                def _():
                    cp_chunk(2, g + 1).start()

            @pl.when(w == 2)
            def _():
                @pl.when(g < NG - 1)
                def _():
                    cp_chunk(0, g + 1).wait()

                cp_wo(g).wait()
                relayout(0, wq_p.at[:, CW:], col)
                for r in range(0, CW, 128):
                    wo_p[r // 2:(r + 128) // 2, pl.ds(pl.multiple_of(col, CW), D)] = (
                        _pk(wo_l[r:r + 128, :]))
                proj_extra(2, col)

                @pl.when(g < NG - 2)
                def _():
                    cp_chunk(0, g + 2).start()

                @pl.when(g < NG - 1)
                def _():
                    cp_wo(g + 1).start()

                @pl.when(g == NG - 2)
                def _():
                    for cp in cp_b_first() + cp_b_rest():
                        cp.start()

            return carry

        lax.fori_loop(1, 3 * NG, chunk_body, 0)
        cp_xf().wait()
        cp_mem().wait()
        for cp in cp_b_first():
            cp.wait()

        scale = E ** -0.5
        zpad = jnp.zeros((LP - L, E), bf16)

        def masks(paired):
            shape = (NR + 2 * NX, 2 * L) if paired else (NR, LP)
            row = lax.broadcasted_iota(jnp.int32, shape, 0)
            col = lax.broadcasted_iota(jnp.int32, shape, 1)
            if not paired:
                return (row < M) | (row >= col), col < L
            prev_q = (row >= NR) & (row < L)
            prev_k = (col >= NR) & (col < NR + L)
            qi = jnp.where(row >= L, row - NX, row)
            kj = jnp.where(col < NR, col, jnp.where(prev_k, col - NR, col - L))
            return (qi < M) | (qi >= kj), prev_q == prev_k

        mask_tab = (masks(False), masks(True))
        DS, DP = 1, 4
        WO_SPLIT = 8
        hs = H // WO_SPLIT

        def ln_fresh(s):
            xf = _ln(x_s[s, 0:NF, :].astype(f32))
            xf = jnp.concatenate([jnp.zeros((M, D), f32), xf], axis=0)
            xn_p[...] = _pk(xf.astype(bf16))

        ln_fresh(0)

        def step(s, mem, prev):
            paired = prev is not None
            allowed, valid = mask_tab[paired]
            kvs = {}
            e0 = pl.multiple_of(s * NX, NX)
            ep = pl.multiple_of(s * NX - NX, 2 * NX) if paired else None
            lhs = _upk(jnp.concatenate([mem, xn_p[M // 2:, :]], axis=0))
            ln_fresh(jnp.minimum(s + 1, NSEG - 1))
            qs, ks, vs, ps, outs, ys = {}, {}, {}, {}, {}, []

            def proj(h):
                qs[h] = _dot(lhs, _upk(wq_p[:, h * E:(h + 1) * E]))
                ks[h] = _dot(lhs, _upk(wk_p[:, h * E:(h + 1) * E]))
                vs[h] = _dot(lhs, _upk(wv_p[:, h * E:(h + 1) * E]))

            def with_extra(cur, j, h, part):
                c0 = part * HE + h * E
                kvs.setdefault(h, {})[j] = cur
                if paired:
                    return jnp.concatenate(
                        [cur, prev[h][j], qkvx_s[pl.ds(ep, 2 * NX), c0:c0 + E]], axis=0)
                return jnp.concatenate([cur, qkvx_s[pl.ds(e0, NX), c0:c0 + E], zpad], axis=0)

            def scores(h):
                k = with_extra(ks[h].astype(bf16), 0, h, 1)
                q = qs[h].astype(bf16)
                if paired:
                    q = jnp.concatenate([q, qkvx_s[pl.ds(ep, 2 * NX), h * E:(h + 1) * E]], axis=0)
                sc = lax.dot_general(q, k, (((1,), (1,)), ((), ())),
                                     preferred_element_type=f32) * scale
                sc = jnp.where(allowed, sc, -1e9)
                sc = jnp.where(valid, sc, -jnp.inf)
                m = jnp.max(sc, axis=-1, keepdims=True)
                p = jnp.exp(sc - m)
                l = jnp.sum(p, axis=-1, keepdims=True)
                r = pl.reciprocal(l, approx=True)
                r = r * (2.0 - l * r)
                ps[h] = (p * r).astype(bf16)

            def pv(h):
                o = _dot(ps[h], with_extra(vs[h].astype(bf16), 1, h, 2))
                if paired:
                    oex_s[pl.ds(ep, 2 * NX), h * E:(h + 1) * E] = o[NR:].astype(bf16)
                outs[h] = o[0:NR].astype(bf16)

            def wo(j):
                oj = jnp.concatenate([outs[h] for h in range(j * hs, (j + 1) * hs)], axis=1)
                g, r = divmod(j * hs * E, CW)
                ys.append(_dot(oj, _upk(wo_p[r // 2:(r + hs * E) // 2, g * D:(g + 1) * D])))

            for t in range(H):
                proj(t)
                if t >= DS:
                    scores(t - DS)
                if t >= DP:
                    pv(t - DP)
            wo(0)
            wo(1)
            scores(H - 1)
            wo(2)
            wo(3)
            pv(H - 4)
            pv(H - 3)
            pv(H - 2)
            wo(4)
            wo(5)
            pv(H - 1)
            wo(6)
            wo(7)
            y = ys[0]
            for yy in ys[1:]:
                y = y + yy
            h_s[s, 0:NF, :] = x_s[s, 0:NF, :].astype(f32) + y[M:]
            return _pk(y[:M].astype(bf16)), kvs

        def wo_extra(grp, c0, n):
            e0 = pl.multiple_of(grp * NR, NR)
            s0 = pl.multiple_of(grp * XG, XG)
            y = None
            for g in range(NG):
                c = pl.multiple_of(g * D + c0, 128)
                yg = _dot(oex_s[pl.ds(e0, NR), g * CW:(g + 1) * CW], _upk(wo_p[:, pl.ds(c, n)]))
                y = yg if y is None else y + yg
            xe = x_s[pl.ds(s0, XG), NF:SEG, pl.ds(c0, n)].astype(f32)
            h_s[pl.ds(s0, XG), NF:SEG, pl.ds(c0, n)] = xe + y.reshape(XG, NX, n)

        oex_s[0:NR, :] = jnp.zeros((NR, HE), bf16)
        HALF = D // 2

        def steps(i, mem):
            @pl.when(i == 1)
            def _():
                for cp in cp_b_rest():
                    cp.wait()

            mem, kvs = step(2 * i, mem, None)
            wo_extra(jnp.maximum(i // 2 - 1, 0), pl.multiple_of((i % 2) * HALF, HALF), HALF)
            mem, _ = step(2 * i + 1, mem, kvs)
            for src, dst, n in zip(b_land, b_pack, b_rows):
                dst[pl.ds(pl.multiple_of(i * (n // 2), n // 2), n // 2), :] = (
                    _pk(src[pl.ds(pl.multiple_of(i * n, n), n), :]))
            return mem

        lax.fori_loop(0, NIT, steps, _pk(mem0_s[...]))
        wo_extra(NSEG // XG - 1, 0, D)

    pl.run_scoped(
        phase_a,
        pltpu.VMEM((D // 2, HE + HG * E), u32),
        pltpu.VMEM((D // 2, HE), u32),
        pltpu.VMEM((D // 2, HE), u32),
        pltpu.VMEM((HG * E, D), bf16),
        pltpu.VMEM((HG * E // 2, NG * D), u32),
        pltpu.VMEM((3, D, HG, E), bf16),
        pltpu.VMEM((D * HG // 2, E), u32),
        pltpu.VMEM((NSEG * NX // 2, D), u32),
        pltpu.VMEM(((M + SEG - NX) // 2, D), u32),
        pltpu.VMEM((NSEG * NX, 3 * HE), bf16),
        pltpu.VMEM((NSEG * NX, HE), bf16),
    )

    NB = S // RB
    bseg = RB // SEG
    cq = D // 4

    def phase_b(g_s, a1_s, a_s, r_s, u_s, o_st):
        g_s[0:8, :] = jnp.zeros((8, D), f32)
        g_s[S + 8:S + 16, :] = jnp.zeros((8, D), f32)

        def load_h(i):
            return h_s[pl.ds(pl.multiple_of(i * bseg, bseg), bseg)].reshape(RB, D)

        def prep(i):
            return _pk(_ln2(load_h(i)).astype(bf16))

        def w1_stage(i):
            a = _upk(a1_s[...])
            r0 = pl.multiple_of(i * RB + 8, 8)
            for c in range(4):
                g = _gelu(_dot(a, _upk(w1_p[:, c * cq:(c + 1) * cq])))
                g_s[pl.ds(r0, RB), c * cq:(c + 1) * cq] = g

        def mix(i):
            r0 = pl.multiple_of(i * RB, RB)
            g0 = g_s[pl.ds(r0, RB + 16), 0 * cq:1 * cq][7:7 + RB]
            g1 = g_s[pl.ds(r0, RB + 16), 1 * cq:2 * cq][9:9 + RB]
            g2 = g_s[pl.ds(r0, RB + 16), 2 * cq:3 * cq][6:6 + RB]
            g3 = g_s[pl.ds(r0, RB + 16), 3 * cq:4 * cq][10:10 + RB]
            gs = jnp.concatenate([g0, g1, g2, g3], axis=1).astype(bf16)
            hsft = _dot(gs, _upk(w2_p[...]))
            hb = load_h(i)
            x1 = _ln(hb) + hsft
            a_s[...] = _pk(_ln(x1).astype(bf16))
            r_s[i % 2] = hb + x1

        def cp_out(i, slot):
            r0 = pl.multiple_of(i * RB, RB)
            return pltpu.make_async_copy(o_st.at[slot], out_hbm.at[pl.ds(r0, RB), :],
                                         sems.at[S_OUT + slot])

        def block(i, slot, with_prep, with_w1, with_mix):
            if with_w1:
                w1_stage(i + 2)
            if with_prep:
                a1_s[...] = prep(i + 3)
            a = _upk(a_s[...])
            for c in range(F // FC):
                u = _dot(a, _upk(w3_p[:, c * FC:(c + 1) * FC]))
                u_s[:, c * FC:(c + 1) * FC] = _pk(_gelu(u).astype(bf16))
            if with_mix:
                mix(i + 1)
            y = _dot(_upk(u_s[...]), _upk(w4_p[...]))
            o_st[slot] = (r_s[slot] + y).astype(bf16)
            cp_out(i, slot).start()

        a1_s[...] = prep(0)
        w1_stage(0)
        a1_s[...] = prep(1)
        w1_stage(1)
        a1_s[...] = prep(2)
        mix(0)

        def body(i, carry, **kw):
            slot = i % 2

            @pl.when(i >= 2)
            def _():
                cp_out(i - 2, slot).wait()

            block(i, slot, **kw)
            return carry

        lax.fori_loop(0, NB - 3, functools.partial(body, with_prep=True, with_w1=True, with_mix=True), 0)
        for i in range(NB - 3, NB):
            cp_out(i - 2, i % 2).wait()
            block(i, i % 2, with_prep=False, with_w1=i + 2 < NB, with_mix=i + 1 < NB)
        cp_out(NB - 2, (NB - 2) % 2).wait()
        cp_out(NB - 1, (NB - 1) % 2).wait()

    pl.run_scoped(
        phase_b,
        pltpu.VMEM((S + 16, D), f32),
        pltpu.VMEM((RB // 2, D), u32),
        pltpu.VMEM((RB // 2, D), u32),
        pltpu.VMEM((2, RB, D), f32),
        pltpu.VMEM((RB // 2, F), u32),
        pltpu.VMEM((2, RB, D), bf16),
    )


@functools.partial(jax.jit, static_argnames=("SEG",))
def _forward(x, mem0, wq, wk, wv, wo, w1, w2, w3, w4, *, SEG):
    B, S, D = x.shape
    _, H, E = wq.shape
    M = mem0.shape[1]
    F = w3.shape[1]
    NSEG = S // SEG
    assert B == 1 and M == 8 and SEG == 32 and E == 128 and S == NSEG * SEG
    assert D == HG * E and H % HG == 0 and H // HG >= 2 and H % 16 == 0
    assert S % RB == 0 and S // RB >= 4 and F % FC == 0
    assert (NSEG * NX) % 256 == 0 and NSEG % 16 == 0
    assert D % (8 * NSEG) == 0 and F % (8 * NSEG) == 0

    hbm = pl.BlockSpec(memory_space=pl.ANY)
    kernel = functools.partial(_kernel, NSEG=NSEG, SEG=SEG, D=D, H=H, E=E, M=M, F=F)
    out = pl.pallas_call(
        kernel,
        out_shape=jax.ShapeDtypeStruct((S, D), x.dtype),
        in_specs=[hbm] * 10,
        out_specs=hbm,
        scratch_shapes=[
            pltpu.VMEM((NSEG, SEG, D), bf16),
            pltpu.VMEM((NSEG, SEG, D), f32),
            pltpu.VMEM((M, D), bf16),
            pltpu.VMEM((D, D), bf16),
            pltpu.VMEM((D, D), bf16),
            pltpu.VMEM((D, F), bf16),
            pltpu.VMEM((F, D), bf16),
            pltpu.VMEM((D // 2, D), u32),
            pltpu.VMEM((D // 2, D), u32),
            pltpu.VMEM((D // 2, F), u32),
            pltpu.VMEM((F // 2, D), u32),
            pltpu.SemaphoreType.DMA((N_SEMS,)),
        ],
        compiler_params=pltpu.CompilerParams(vmem_limit_bytes=124 * 1024 * 1024),
        name="rmt_mixer",
    )(
        x.reshape(NSEG, SEG, D),
        mem0.reshape(M, D),
        wq, wk, wv,
        wo.reshape(H * E, D),
        w1, w2, w3, w4,
    )
    return out.reshape(B, S, D)


def pallas_sequential_preLN__memory_aug_recurrent_mem_tr__mixer_s_mlp__prompt_kernel(
    A_x, A_mem0, A_Wq, A_Wk, A_Wv, A_Wo, A_seg_len, B_x, B_w1, B_w2, B_w3, B_w4
):
    del B_x
    seg = A_seg_len if isinstance(A_seg_len, int) else 32
    return _forward(A_x, A_mem0, A_Wq, A_Wk, A_Wv, A_Wo, B_w1, B_w2, B_w3, B_w4, SEG=seg)
```

```python
import functools

import jax
import jax.numpy as jnp
from jax import lax
from jax.experimental import pallas as pl
from jax.experimental.pallas import tpu as pltpu

bf16, f32, u32 = jnp.bfloat16, jnp.float32, jnp.uint32

LN_EPS = 1e-5
NX = 8
HG = 8
RB = 128
FC = 512

S_XE, S_XF, S_LAND, S_WO, S_MEM, S_B0, S_B1, S_OUT = 0, 2, 3, 6, 7, 8, 12, 16
N_SEMS = 18


def _pk(x):
    return pltpu.bitcast(x, u32)


def _upk(x):
    return pltpu.bitcast(x, bf16)


def _dot(a, b):
    return jnp.dot(a, b, preferred_element_type=f32)


def _ln(x):
    m = jnp.mean(x, axis=-1, keepdims=True)
    xc = x - m
    v = jnp.mean(xc * xc, axis=-1, keepdims=True)
    return xc * lax.rsqrt(v + LN_EPS)


def _ln2(x):
    m = jnp.mean(x, axis=-1, keepdims=True)
    xc = x - m
    v = jnp.mean(xc * xc, axis=-1, keepdims=True)
    r = lax.rsqrt(v + LN_EPS)
    return xc * (r * lax.rsqrt(v * (r * r) + LN_EPS))


def _gelu(x):
    c = 0.7978845608028654
    return x * (0.5 + 0.5 * jnp.tanh(x * (c + (c * 0.044715) * (x * x))))


def _kernel(x_hbm, mem0_hbm, wq_hbm, wk_hbm, wv_hbm, wo_hbm, w1_hbm, w2_hbm, w3_hbm, w4_hbm,
            out_hbm,
            x_s, h_s, mem0_s, w1_l, w2_l, w3_l, w4_l, w1_p, w2_p, w3_p, w4_p, sems,
            *, NSEG, SEG, D, H, E, M, F):
    S = NSEG * SEG
    NF = SEG - NX
    NR = M + NF
    L = M + SEG
    LP = L + 8
    HE = H * E
    NG = H // HG
    w_hbm = (wq_hbm, wk_hbm, wv_hbm)

    def cp_xe(half):
        s0, s1 = half * NSEG // 2, (half + 1) * NSEG // 2
        return pltpu.make_async_copy(x_hbm.at[s0:s1, NF:SEG, :], x_s.at[s0:s1, NF:SEG, :],
                                     sems.at[S_XE + half])

    XG = (M + SEG - NX) // NX
    NIT = NSEG // 2
    b_hbm = (w1_hbm, w2_hbm, w3_hbm, w4_hbm)
    b_land = (w1_l, w2_l, w3_l, w4_l)
    b_pack = (w1_p, w2_p, w3_p, w4_p)
    b_rows = tuple(r.shape[0] // NIT for r in b_hbm)

    def cp_b_first():
        return [pltpu.make_async_copy(h.at[0:n], l.at[0:n], sems.at[S_B0 + j])
                for j, (h, l, n) in enumerate(zip(b_hbm, b_land, b_rows))]

    def cp_b_rest():
        return [pltpu.make_async_copy(h.at[n:], l.at[n:], sems.at[S_B1 + j])
                for j, (h, l, n) in enumerate(zip(b_hbm, b_land, b_rows))]

    def cp_mem():
        return pltpu.make_async_copy(mem0_hbm, mem0_s, sems.at[S_MEM])

    def phase_a(wq_p, wk_p, wv_p, wo_l, wo_p, land, stage, xe_p, xn_p, qkvx_s, oex_s):
        w_p = (wq_p, wk_p, wv_p)
        CW = HG * E

        def cp_chunk(w, g):
            g0 = pl.multiple_of(g * HG, HG)
            return pltpu.make_async_copy(w_hbm[w].at[:, pl.ds(g0, HG), :], land.at[w],
                                         sems.at[S_LAND + w])

        def cp_wo(g):
            r0 = pl.multiple_of(g * CW, CW)
            return pltpu.make_async_copy(wo_hbm.at[pl.ds(r0, CW), :], wo_l, sems.at[S_WO])

        def relayout(w, dst, col0):
            db = 64
            for d0 in range(0, D, db):
                stage[d0 * 4:(d0 + db) * 4, :] = _pk(land[w, d0:d0 + db].reshape(db * HG, E))
            for p in range(HG // 2):
                for d0 in range(0, D, 128):
                    u = stage[pl.ds(d0 * 4 + p, 128, stride=4), :]
                    lo = pltpu.bitcast(u << 16, f32).astype(bf16)
                    hi = pltpu.bitcast(u & jnp.uint32(0xFFFF0000), f32).astype(bf16)
                    c_lo = pl.multiple_of(col0 + (2 * p) * E, E)
                    c_hi = pl.multiple_of(col0 + (2 * p + 1) * E, E)
                    dst[d0 // 2:d0 // 2 + 64, pl.ds(c_lo, E)] = _pk(lo)
                    dst[d0 // 2:d0 // 2 + 64, pl.ds(c_hi, E)] = _pk(hi)

        def proj_extra(w, col0):
            nb = 512
            for mb in range(NSEG * NX // 256):
                a = _upk(xe_p[mb * 128:(mb + 1) * 128, :])
                for nc in range(HG * E // nb):
                    c = pl.multiple_of(col0 + nc * nb, nb)
                    r = _dot(a, _upk(w_p[w][:, pl.ds(c, nb)]))
                    qkvx_s.at[:, w * HE:(w + 1) * HE][mb * 256:(mb + 1) * 256, pl.ds(c, nb)] = (
                        r.astype(bf16))

        def cp_xf():
            return pltpu.make_async_copy(x_hbm.at[:, 0:NF, :], x_s.at[:, 0:NF, :], sems.at[S_XF])

        cp_xe(0).start()
        cp_chunk(0, 0).start()
        cp_xe(1).start()
        cp_chunk(1, 0).start()
        cp_chunk(2, 0).start()
        cp_mem().start()
        cp_wo(0).start()

        def ln_extra(half):
            sb = 16
            for s0 in range(half * NSEG // 2, (half + 1) * NSEG // 2, sb):
                xe = x_s[s0:s0 + sb, NF:SEG, :].astype(f32).reshape(sb * NX, D)
                xe_p[s0 * NX // 2:(s0 + sb) * NX // 2, :] = _pk(_ln(xe).astype(bf16))

        cp_xe(0).wait()
        ln_extra(0)
        cp_chunk(0, 0).wait()
        relayout(0, wq_p, 0)
        cp_chunk(0, 1).start()
        cp_xe(1).wait()
        ln_extra(1)
        proj_extra(0, 0)
        cp_chunk(1, 0).wait()
        relayout(1, wk_p, 0)
        cp_chunk(1, 1).start()

        def chunk_body(c, carry):
            g = c // 3
            w = c - 3 * g
            col = g * CW

            @pl.when(w == 0)
            def _():
                cp_chunk(1, g).wait()
                relayout(1, wk_p, col)
                proj_extra(0, col)

                @pl.when(g < NG - 1)
                def _():
                    cp_chunk(1, g + 1).start()

                @pl.when(g == 1)
                def _():
                    cp_xf().start()

            @pl.when(w == 1)
            def _():
                cp_chunk(2, g).wait()
                relayout(2, wv_p, col)
                proj_extra(1, col)

                @pl.when(g < NG - 1)
                def _():
                    cp_chunk(2, g + 1).start()

            @pl.when(w == 2)
            def _():
                @pl.when(g < NG - 1)
                def _():
                    cp_chunk(0, g + 1).wait()

                cp_wo(g).wait()
                relayout(0, wq_p.at[:, CW:], col)
                for r in range(0, CW, 128):
                    wo_p[r // 2:(r + 128) // 2, pl.ds(pl.multiple_of(col, CW), D)] = (
                        _pk(wo_l[r:r + 128, :]))
                proj_extra(2, col)

                @pl.when(g < NG - 2)
                def _():
                    cp_chunk(0, g + 2).start()

                @pl.when(g < NG - 1)
                def _():
                    cp_wo(g + 1).start()

                @pl.when(g == NG - 2)
                def _():
                    for cp in cp_b_first() + cp_b_rest():
                        cp.start()

            return carry

        lax.fori_loop(1, 3 * NG, chunk_body, 0)
        cp_xf().wait()
        cp_mem().wait()
        for cp in cp_b_first():
            cp.wait()

        scale = E ** -0.5
        zpad = jnp.zeros((LP - L, E), bf16)

        def masks(paired):
            shape = (NR + 2 * NX, 2 * L) if paired else (NR, LP)
            row = lax.broadcasted_iota(jnp.int32, shape, 0)
            col = lax.broadcasted_iota(jnp.int32, shape, 1)
            if not paired:
                return (row < M) | (row >= col), col < L
            prev_q = (row >= NR) & (row < L)
            prev_k = (col >= NR) & (col < NR + L)
            qi = jnp.where(row >= L, row - NX, row)
            kj = jnp.where(col < NR, col, jnp.where(prev_k, col - NR, col - L))
            return (qi < M) | (qi >= kj), prev_q == prev_k

        mask_tab = (masks(False), masks(True))
        DS, DP = 1, 4
        WO_SPLIT = 8
        hs = H // WO_SPLIT

        def ln_fresh(s):
            xf = _ln(x_s[s, 0:NF, :].astype(f32))
            xf = jnp.concatenate([jnp.zeros((M, D), f32), xf], axis=0)
            xn_p[...] = _pk(xf.astype(bf16))

        ln_fresh(0)

        def step(s, mem, prev):
            paired = prev is not None
            allowed, valid = mask_tab[paired]
            kvs = {}
            e0 = pl.multiple_of(s * NX, NX)
            ep = pl.multiple_of(s * NX - NX, 2 * NX) if paired else None
            lhs = _upk(jnp.concatenate([mem, xn_p[M // 2:, :]], axis=0))
            ln_fresh(jnp.minimum(s + 1, NSEG - 1))
            qs, ks, vs, ps, outs, ys = {}, {}, {}, {}, {}, []

            def proj(h):
                qs[h] = _dot(lhs, _upk(wq_p[:, h * E:(h + 1) * E]))
                ks[h] = _dot(lhs, _upk(wk_p[:, h * E:(h + 1) * E]))
                vs[h] = _dot(lhs, _upk(wv_p[:, h * E:(h + 1) * E]))

            def with_extra(cur, j, h, part):
                c0 = part * HE + h * E
                kvs.setdefault(h, {})[j] = cur
                if paired:
                    return jnp.concatenate(
                        [cur, prev[h][j], qkvx_s[pl.ds(ep, 2 * NX), c0:c0 + E]], axis=0)
                return jnp.concatenate([cur, qkvx_s[pl.ds(e0, NX), c0:c0 + E], zpad], axis=0)

            def scores(h):
                k = with_extra(ks[h].astype(bf16), 0, h, 1)
                q = qs[h].astype(bf16)
                if paired:
                    q = jnp.concatenate([q, qkvx_s[pl.ds(ep, 2 * NX), h * E:(h + 1) * E]], axis=0)
                sc = lax.dot_general(q, k, (((1,), (1,)), ((), ())),
                                     preferred_element_type=f32) * scale
                sc = jnp.where(allowed, sc, -1e9)
                sc = jnp.where(valid, sc, -jnp.inf)
                m = jnp.max(sc, axis=-1, keepdims=True)
                p = jnp.exp(sc - m)
                l = jnp.sum(p, axis=-1, keepdims=True)
                r = pl.reciprocal(l, approx=True)
                r = r * (2.0 - l * r)
                ps[h] = (p * r).astype(bf16)

            def pv(h):
                o = _dot(ps[h], with_extra(vs[h].astype(bf16), 1, h, 2))
                if paired:
                    oex_s[pl.ds(ep, 2 * NX), h * E:(h + 1) * E] = o[NR:].astype(bf16)
                outs[h] = o[0:NR].astype(bf16)

            def wo(j):
                oj = jnp.concatenate([outs[h] for h in range(j * hs, (j + 1) * hs)], axis=1)
                g, r = divmod(j * hs * E, CW)
                ys.append(_dot(oj, _upk(wo_p[r // 2:(r + hs * E) // 2, g * D:(g + 1) * D])))

            for t in range(H):
                proj(t)
                if t >= DS:
                    scores(t - DS)
                if t >= DP:
                    pv(t - DP)
            wo(0)
            wo(1)
            scores(H - 1)
            wo(2)
            wo(3)
            pv(H - 4)
            pv(H - 3)
            pv(H - 2)
            wo(4)
            wo(5)
            pv(H - 1)
            wo(6)
            wo(7)
            y = ys[0]
            for yy in ys[1:]:
                y = y + yy
            h_s[s, 0:NF, :] = x_s[s, 0:NF, :].astype(f32) + y[M:]
            return _pk(y[:M].astype(bf16)), kvs

        def wo_extra(grp, c0, n):
            e0 = pl.multiple_of(grp * NR, NR)
            s0 = pl.multiple_of(grp * XG, XG)
            y = None
            for g in range(NG):
                c = pl.multiple_of(g * D + c0, 128)
                yg = _dot(oex_s[pl.ds(e0, NR), g * CW:(g + 1) * CW], _upk(wo_p[:, pl.ds(c, n)]))
                y = yg if y is None else y + yg
            xe = x_s[pl.ds(s0, XG), NF:SEG, pl.ds(c0, n)].astype(f32)
            h_s[pl.ds(s0, XG), NF:SEG, pl.ds(c0, n)] = xe + y.reshape(XG, NX, n)

        oex_s[0:NR, :] = jnp.zeros((NR, HE), bf16)
        HALF = D // 2

        def steps(i, mem):
            @pl.when(i == 1)
            def _():
                for cp in cp_b_rest():
                    cp.wait()

            mem, kvs = step(2 * i, mem, None)
            wo_extra(jnp.maximum(i // 2 - 1, 0), pl.multiple_of((i % 2) * HALF, HALF), HALF)
            mem, _ = step(2 * i + 1, mem, kvs)
            for src, dst, n in zip(b_land, b_pack, b_rows):
                dst[pl.ds(pl.multiple_of(i * (n // 2), n // 2), n // 2), :] = (
                    _pk(src[pl.ds(pl.multiple_of(i * n, n), n), :]))
            return mem

        lax.fori_loop(0, NIT, steps, _pk(mem0_s[...]))
        wo_extra(NSEG // XG - 1, 0, D)

    pl.run_scoped(
        phase_a,
        pltpu.VMEM((D // 2, HE + HG * E), u32),
        pltpu.VMEM((D // 2, HE), u32),
        pltpu.VMEM((D // 2, HE), u32),
        pltpu.VMEM((HG * E, D), bf16),
        pltpu.VMEM((HG * E // 2, NG * D), u32),
        pltpu.VMEM((3, D, HG, E), bf16),
        pltpu.VMEM((D * HG // 2, E), u32),
        pltpu.VMEM((NSEG * NX // 2, D), u32),
        pltpu.VMEM(((M + SEG - NX) // 2, D), u32),
        pltpu.VMEM((NSEG * NX, 3 * HE), bf16),
        pltpu.VMEM((NSEG * NX, HE), bf16),
    )

    NB = S // RB
    bseg = RB // SEG
    cq = D // 4

    def phase_b(g_s, a1_s, a_s, r_s, u_s, o_st):
        g_s[0:8, :] = jnp.zeros((8, D), f32)
        g_s[S + 8:S + 16, :] = jnp.zeros((8, D), f32)

        def load_h(i):
            return h_s[pl.ds(pl.multiple_of(i * bseg, bseg), bseg)].reshape(RB, D)

        def prep(i):
            return _pk(_ln2(load_h(i)).astype(bf16))

        def w1_stage(i):
            a = _upk(a1_s[...])
            r0 = pl.multiple_of(i * RB + 8, 8)
            for c in range(4):
                g = _gelu(_dot(a, _upk(w1_p[:, c * cq:(c + 1) * cq])))
                g_s[pl.ds(r0, RB), c * cq:(c + 1) * cq] = g

        def mix(i):
            r0 = pl.multiple_of(i * RB, RB)
            g0 = g_s[pl.ds(r0, RB + 16), 0 * cq:1 * cq][7:7 + RB]
            g1 = g_s[pl.ds(r0, RB + 16), 1 * cq:2 * cq][9:9 + RB]
            g2 = g_s[pl.ds(r0, RB + 16), 2 * cq:3 * cq][6:6 + RB]
            g3 = g_s[pl.ds(r0, RB + 16), 3 * cq:4 * cq][10:10 + RB]
            gs = jnp.concatenate([g0, g1, g2, g3], axis=1).astype(bf16)
            hsft = _dot(gs, _upk(w2_p[...]))
            hb = load_h(i)
            x1 = _ln(hb) + hsft
            a_s[...] = _pk(_ln(x1).astype(bf16))
            r_s[i % 2] = hb + x1

        def cp_out(i, slot):
            r0 = pl.multiple_of(i * RB, RB)
            return pltpu.make_async_copy(o_st.at[slot], out_hbm.at[pl.ds(r0, RB), :],
                                         sems.at[S_OUT + slot])

        def block(i, slot, with_prep, with_w1, with_mix):
            if with_w1:
                w1_stage(i + 2)
            if with_prep:
                a1_s[...] = prep(i + 3)
            a = _upk(a_s[...])
            for c in range(F // FC):
                u = _dot(a, _upk(w3_p[:, c * FC:(c + 1) * FC]))
                u_s[:, c * FC:(c + 1) * FC] = _pk(_gelu(u).astype(bf16))
            if with_mix:
                mix(i + 1)
            y = _dot(_upk(u_s[...]), _upk(w4_p[...]))
            o_st[slot] = (r_s[slot] + y).astype(bf16)
            cp_out(i, slot).start()

        a1_s[...] = prep(0)
        w1_stage(0)
        a1_s[...] = prep(1)
        w1_stage(1)
        a1_s[...] = prep(2)
        mix(0)

        def body(i, carry, **kw):
            slot = i % 2

            @pl.when(i >= 2)
            def _():
                cp_out(i - 2, slot).wait()

            block(i, slot, **kw)
            return carry

        lax.fori_loop(0, NB - 3, functools.partial(body, with_prep=True, with_w1=True, with_mix=True), 0)
        for i in range(NB - 3, NB):
            cp_out(i - 2, i % 2).wait()
            block(i, i % 2, with_prep=False, with_w1=i + 2 < NB, with_mix=i + 1 < NB)
        cp_out(NB - 2, (NB - 2) % 2).wait()
        cp_out(NB - 1, (NB - 1) % 2).wait()

    pl.run_scoped(
        phase_b,
        pltpu.VMEM((S + 16, D), f32),
        pltpu.VMEM((RB // 2, D), u32),
        pltpu.VMEM((RB // 2, D), u32),
        pltpu.VMEM((2, RB, D), f32),
        pltpu.VMEM((RB // 2, F), u32),
        pltpu.VMEM((2, RB, D), bf16),
    )


@functools.partial(jax.jit, static_argnames=("SEG",))
def _forward(x, mem0, wq, wk, wv, wo, w1, w2, w3, w4, *, SEG):
    B, S, D = x.shape
    _, H, E = wq.shape
    M = mem0.shape[1]
    F = w3.shape[1]
    NSEG = S // SEG
    assert B == 1 and M == 8 and SEG == 32 and E == 128 and S == NSEG * SEG
    assert D == HG * E and H % HG == 0 and H // HG >= 2 and H % 16 == 0
    assert S % RB == 0 and S // RB >= 4 and F % FC == 0
    assert (NSEG * NX) % 256 == 0 and NSEG % 32 == 0
    assert D % (8 * NSEG) == 0 and F % (8 * NSEG) == 0

    hbm = pl.BlockSpec(memory_space=pl.ANY)
    kernel = functools.partial(_kernel, NSEG=NSEG, SEG=SEG, D=D, H=H, E=E, M=M, F=F)
    out = pl.pallas_call(
        kernel,
        out_shape=jax.ShapeDtypeStruct((S, D), x.dtype),
        in_specs=[hbm] * 10,
        out_specs=hbm,
        scratch_shapes=[
            pltpu.VMEM((NSEG, SEG, D), bf16),
            pltpu.VMEM((NSEG, SEG, D), f32),
            pltpu.VMEM((M, D), bf16),
            pltpu.VMEM((D, D), bf16),
            pltpu.VMEM((D, D), bf16),
            pltpu.VMEM((D, F), bf16),
            pltpu.VMEM((F, D), bf16),
            pltpu.VMEM((D // 2, D), u32),
            pltpu.VMEM((D // 2, D), u32),
            pltpu.VMEM((D // 2, F), u32),
            pltpu.VMEM((F // 2, D), u32),
            pltpu.SemaphoreType.DMA((N_SEMS,)),
        ],
        compiler_params=pltpu.CompilerParams(vmem_limit_bytes=124 * 1024 * 1024),
        name="rmt_mixer",
    )(
        x.reshape(NSEG, SEG, D),
        mem0.reshape(M, D),
        wq, wk, wv,
        wo.reshape(H * E, D),
        w1, w2, w3, w4,
    )
    return out.reshape(B, S, D)


def pallas_sequential_preLN__memory_aug_recurrent_mem_tr__mixer_s_mlp__prompt_kernel(
    A_x, A_mem0, A_Wq, A_Wk, A_Wv, A_Wo, A_seg_len, B_x, B_w1, B_w2, B_w3, B_w4
):
    del B_x
    seg = A_seg_len if isinstance(A_seg_len, int) else 32
    return _forward(A_x, A_mem0, A_Wq, A_Wk, A_Wv, A_Wo, B_w1, B_w2, B_w3, B_w4, SEG=seg)
```

```python
import functools

import jax
import jax.numpy as jnp
from jax import lax
from jax.experimental import pallas as pl
from jax.experimental.pallas import tpu as pltpu

bf16, f32, u32 = jnp.bfloat16, jnp.float32, jnp.uint32

LN_EPS = 1e-5
NX = 8
HG = 8
RB = 128
FC = 512

S_XE, S_XF, S_LAND, S_WO, S_MEM, S_B0, S_B1, S_OUT = 0, 2, 3, 6, 7, 8, 12, 16
N_SEMS = 18


def _pk(x):
    return pltpu.bitcast(x, u32)


def _upk(x):
    return pltpu.bitcast(x, bf16)


def _dot(a, b):
    return jnp.dot(a, b, preferred_element_type=f32)


def _ln(x):
    m = jnp.mean(x, axis=-1, keepdims=True)
    xc = x - m
    v = jnp.mean(xc * xc, axis=-1, keepdims=True)
    return xc * lax.rsqrt(v + LN_EPS)


def _ln2(x):
    m = jnp.mean(x, axis=-1, keepdims=True)
    xc = x - m
    v = jnp.mean(xc * xc, axis=-1, keepdims=True)
    r = lax.rsqrt(v + LN_EPS)
    return xc * (r * lax.rsqrt(v * (r * r) + LN_EPS))


def _gelu(x):
    c = 0.7978845608028654
    return x * (0.5 + 0.5 * jnp.tanh(x * (c + (c * 0.044715) * (x * x))))


def _kernel(x_hbm, mem0_hbm, wq_hbm, wk_hbm, wv_hbm, wo_hbm, w1_hbm, w2_hbm, w3_hbm, w4_hbm,
            out_hbm,
            x_s, h_s, mem0_s, w1_l, w2_l, w3_l, w4_l, w1_p, w2_p, w3_p, w4_p, sems,
            *, NSEG, SEG, D, H, E, M, F):
    S = NSEG * SEG
    NF = SEG - NX
    NR = M + NF
    L = M + SEG
    LP = L + 8
    HE = H * E
    NG = H // HG
    w_hbm = (wq_hbm, wk_hbm, wv_hbm)

    def cp_xe(half):
        s0, s1 = half * NSEG // 2, (half + 1) * NSEG // 2
        return pltpu.make_async_copy(x_hbm.at[s0:s1, NF:SEG, :], x_s.at[s0:s1, NF:SEG, :],
                                     sems.at[S_XE + half])

    XG = (M + SEG - NX) // NX
    NIT = NSEG // 2
    b_hbm = (w1_hbm, w2_hbm, w3_hbm, w4_hbm)
    b_land = (w1_l, w2_l, w3_l, w4_l)
    b_pack = (w1_p, w2_p, w3_p, w4_p)
    b_rows = tuple(r.shape[0] // NIT for r in b_hbm)

    def cp_b_first():
        return [pltpu.make_async_copy(h.at[0:n], l.at[0:n], sems.at[S_B0 + j])
                for j, (h, l, n) in enumerate(zip(b_hbm, b_land, b_rows))]

    def cp_b_rest():
        return [pltpu.make_async_copy(h.at[n:], l.at[n:], sems.at[S_B1 + j])
                for j, (h, l, n) in enumerate(zip(b_hbm, b_land, b_rows))]

    def cp_mem():
        return pltpu.make_async_copy(mem0_hbm, mem0_s, sems.at[S_MEM])

    def phase_a(wq_p, wk_p, wv_p, wo_l, wo_p, land, stage, xe_p, xn_p, qkvx_s, oex_s):
        w_p = (wq_p, wk_p, wv_p)
        CW = HG * E

        def cp_chunk(w, g):
            g0 = pl.multiple_of(g * HG, HG)
            return pltpu.make_async_copy(w_hbm[w].at[:, pl.ds(g0, HG), :], land.at[w],
                                         sems.at[S_LAND + w])

        def cp_wo(g):
            r0 = pl.multiple_of(g * CW, CW)
            return pltpu.make_async_copy(wo_hbm.at[pl.ds(r0, CW), :], wo_l, sems.at[S_WO])

        def relayout(w, dst, col0):
            db = 64
            for d0 in range(0, D, db):
                stage[d0 * 4:(d0 + db) * 4, :] = _pk(land[w, d0:d0 + db].reshape(db * HG, E))
            for p in range(HG // 2):
                for d0 in range(0, D, 128):
                    u = stage[pl.ds(d0 * 4 + p, 128, stride=4), :]
                    lo = pltpu.bitcast(u << 16, f32).astype(bf16)
                    hi = pltpu.bitcast(u & jnp.uint32(0xFFFF0000), f32).astype(bf16)
                    c_lo = pl.multiple_of(col0 + (2 * p) * E, E)
                    c_hi = pl.multiple_of(col0 + (2 * p + 1) * E, E)
                    dst[d0 // 2:d0 // 2 + 64, pl.ds(c_lo, E)] = _pk(lo)
                    dst[d0 // 2:d0 // 2 + 64, pl.ds(c_hi, E)] = _pk(hi)

        def proj_extra(w, col0):
            nb = 512
            for mb in range(NSEG * NX // 256):
                a = _upk(xe_p[mb * 128:(mb + 1) * 128, :])
                for nc in range(HG * E // nb):
                    c = pl.multiple_of(col0 + nc * nb, nb)
                    r = _dot(a, _upk(w_p[w][:, pl.ds(c, nb)]))
                    qkvx_s.at[:, w * HE:(w + 1) * HE][mb * 256:(mb + 1) * 256, pl.ds(c, nb)] = (
                        r.astype(bf16))

        def cp_xf():
            return pltpu.make_async_copy(x_hbm.at[:, 0:NF, :], x_s.at[:, 0:NF, :], sems.at[S_XF])

        cp_xe(0).start()
        cp_chunk(0, 0).start()
        cp_xe(1).start()
        cp_chunk(1, 0).start()
        cp_chunk(2, 0).start()
        cp_mem().start()
        cp_wo(0).start()

        def ln_extra(half):
            sb = 16
            for s0 in range(half * NSEG // 2, (half + 1) * NSEG // 2, sb):
                xe = x_s[s0:s0 + sb, NF:SEG, :].astype(f32).reshape(sb * NX, D)
                xe_p[s0 * NX // 2:(s0 + sb) * NX // 2, :] = _pk(_ln(xe).astype(bf16))

        cp_xe(0).wait()
        ln_extra(0)
        cp_chunk(0, 0).wait()
        relayout(0, wq_p, 0)
        cp_chunk(0, 1).start()
        cp_xe(1).wait()
        ln_extra(1)
        proj_extra(0, 0)
        cp_chunk(1, 0).wait()
        relayout(1, wk_p, 0)
        cp_chunk(1, 1).start()

        def chunk_body(c, carry):
            g = c // 3
            w = c - 3 * g
            col = g * CW

            @pl.when(w == 0)
            def _():
                cp_chunk(1, g).wait()
                relayout(1, wk_p, col)
                proj_extra(0, col)

                @pl.when(g < NG - 1)
                def _():
                    cp_chunk(1, g + 1).start()

                @pl.when(g == 1)
                def _():
                    cp_xf().start()

            @pl.when(w == 1)
            def _():
                cp_chunk(2, g).wait()
                relayout(2, wv_p, col)
                proj_extra(1, col)

                @pl.when(g < NG - 1)
                def _():
                    cp_chunk(2, g + 1).start()

            @pl.when(w == 2)
            def _():
                @pl.when(g < NG - 1)
                def _():
                    cp_chunk(0, g + 1).wait()

                cp_wo(g).wait()
                relayout(0, wq_p.at[:, CW:], col)
                for r in range(0, CW, 128):
                    wo_p[r // 2:(r + 128) // 2, pl.ds(pl.multiple_of(col, CW), D)] = (
                        _pk(wo_l[r:r + 128, :]))
                proj_extra(2, col)

                @pl.when(g < NG - 2)
                def _():
                    cp_chunk(0, g + 2).start()

                @pl.when(g < NG - 1)
                def _():
                    cp_wo(g + 1).start()

                @pl.when(g == NG - 2)
                def _():
                    for cp in cp_b_first() + cp_b_rest():
                        cp.start()

            return carry

        lax.fori_loop(1, 3 * NG, chunk_body, 0)
        cp_xf().wait()
        cp_mem().wait()
        for cp in cp_b_first():
            cp.wait()

        scale = E ** -0.5
        zpad = jnp.zeros((LP - L, E), bf16)

        def masks(paired):
            shape = (NR + 2 * NX, 2 * L) if paired else (NR, LP)
            row = lax.broadcasted_iota(jnp.int32, shape, 0)
            col = lax.broadcasted_iota(jnp.int32, shape, 1)
            if not paired:
                return (row < M) | (row >= col), col < L
            prev_q = (row >= NR) & (row < L)
            prev_k = (col >= NR) & (col < NR + L)
            qi = jnp.where(row >= L, row - NX, row)
            kj = jnp.where(col < NR, col, jnp.where(prev_k, col - NR, col - L))
            return (qi < M) | (qi >= kj), prev_q == prev_k

        mask_tab = (masks(False), masks(True))
        DS, DP = 1, 4
        WO_SPLIT = 8
        hs = H // WO_SPLIT

        def ln_fresh(s):
            xf = _ln(x_s[s, 0:NF, :].astype(f32))
            xf = jnp.concatenate([jnp.zeros((M, D), f32), xf], axis=0)
            xn_p[...] = _pk(xf.astype(bf16))

        ln_fresh(0)

        def step(s, mem, prev, ex):
            paired = prev is not None
            allowed, valid = mask_tab[paired]
            kvs = {}
            ep = pl.multiple_of(s * NX - NX, 2 * NX) if paired else None
            lhs = _upk(jnp.concatenate([mem, xn_p[M // 2:, :]], axis=0))
            ln_fresh(jnp.minimum(s + 1, NSEG - 1))
            qs, ks, vs, ps, outs, ys = {}, {}, {}, {}, {}, []

            def proj(h):
                qs[h] = _dot(lhs, _upk(wq_p[:, h * E:(h + 1) * E]))
                ks[h] = _dot(lhs, _upk(wk_p[:, h * E:(h + 1) * E]))
                vs[h] = _dot(lhs, _upk(wv_p[:, h * E:(h + 1) * E]))

            def with_extra(cur, j, h, part):
                c0 = part * HE + h * E
                kvs.setdefault(h, {})[j] = cur
                if paired:
                    return jnp.concatenate([cur, prev[h][j], ex[:, c0:c0 + E]], axis=0)
                return jnp.concatenate([cur, ex[0:NX, c0:c0 + E], zpad], axis=0)

            def scores(h):
                k = with_extra(ks[h].astype(bf16), 0, h, 1)
                q = qs[h].astype(bf16)
                if paired:
                    q = jnp.concatenate([q, ex[:, h * E:(h + 1) * E]], axis=0)
                sc = lax.dot_general(q, k, (((1,), (1,)), ((), ())),
                                     preferred_element_type=f32) * scale
                sc = jnp.where(allowed, sc, -1e9)
                sc = jnp.where(valid, sc, -jnp.inf)
                m = jnp.max(sc, axis=-1, keepdims=True)
                p = jnp.exp(sc - m)
                l = jnp.sum(p, axis=-1, keepdims=True)
                r = pl.reciprocal(l, approx=True)
                r = r * (2.0 - l * r)
                ps[h] = (p * r).astype(bf16)

            def pv(h):
                o = _dot(ps[h], with_extra(vs[h].astype(bf16), 1, h, 2))
                if paired:
                    oex_s[pl.ds(ep, 2 * NX), h * E:(h + 1) * E] = o[NR:].astype(bf16)
                outs[h] = o[0:NR].astype(bf16)

            def wo(j):
                oj = jnp.concatenate([outs[h] for h in range(j * hs, (j + 1) * hs)], axis=1)
                g, r = divmod(j * hs * E, CW)
                ys.append(_dot(oj, _upk(wo_p[r // 2:(r + hs * E) // 2, g * D:(g + 1) * D])))

            for t in range(H):
                proj(t)
                if t >= DS:
                    scores(t - DS)
                if t >= DP:
                    pv(t - DP)
            wo(0)
            wo(1)
            scores(H - 1)
            wo(2)
            wo(3)
            pv(H - 4)
            pv(H - 3)
            pv(H - 2)
            wo(4)
            wo(5)
            pv(H - 1)
            wo(6)
            wo(7)
            y = ys[0]
            for yy in ys[1:]:
                y = y + yy
            h_s[s, 0:NF, :] = x_s[s, 0:NF, :].astype(f32) + y[M:]
            return _pk(y[:M].astype(bf16)), kvs

        def wo_extra(grp, c0, n):
            e0 = pl.multiple_of(grp * NR, NR)
            s0 = pl.multiple_of(grp * XG, XG)
            y = None
            for g in range(NG):
                c = pl.multiple_of(g * D + c0, 128)
                yg = _dot(oex_s[pl.ds(e0, NR), g * CW:(g + 1) * CW], _upk(wo_p[:, pl.ds(c, n)]))
                y = yg if y is None else y + yg
            xe = x_s[pl.ds(s0, XG), NF:SEG, pl.ds(c0, n)].astype(f32)
            h_s[pl.ds(s0, XG), NF:SEG, pl.ds(c0, n)] = xe + y.reshape(XG, NX, n)

        oex_s[0:NR, :] = jnp.zeros((NR, HE), bf16)
        HALF = D // 2

        def steps(i, mem):
            @pl.when(i == 1)
            def _():
                for cp in cp_b_rest():
                    cp.wait()

            ex = qkvx_s[pl.ds(pl.multiple_of(i * 2 * NX, 2 * NX), 2 * NX), :]
            mem, kvs = step(2 * i, mem, None, ex)
            wo_extra(jnp.maximum(i // 2 - 1, 0), pl.multiple_of((i % 2) * HALF, HALF), HALF)
            mem, _ = step(2 * i + 1, mem, kvs, ex)
            for src, dst, n in zip(b_land, b_pack, b_rows):
                dst[pl.ds(pl.multiple_of(i * (n // 2), n // 2), n // 2), :] = (
                    _pk(src[pl.ds(pl.multiple_of(i * n, n), n), :]))
            return mem

        lax.fori_loop(0, NIT, steps, _pk(mem0_s[...]))
        wo_extra(NSEG // XG - 1, 0, D)

    pl.run_scoped(
        phase_a,
        pltpu.VMEM((D // 2, HE + HG * E), u32),
        pltpu.VMEM((D // 2, HE), u32),
        pltpu.VMEM((D // 2, HE), u32),
        pltpu.VMEM((HG * E, D), bf16),
        pltpu.VMEM((HG * E // 2, NG * D), u32),
        pltpu.VMEM((3, D, HG, E), bf16),
        pltpu.VMEM((D * HG // 2, E), u32),
        pltpu.VMEM((NSEG * NX // 2, D), u32),
        pltpu.VMEM(((M + SEG - NX) // 2, D), u32),
        pltpu.VMEM((NSEG * NX, 3 * HE), bf16),
        pltpu.VMEM((NSEG * NX, HE), bf16),
    )

    NB = S // RB
    bseg = RB // SEG
    cq = D // 4

    def phase_b(g_s, a1_s, a_s, r_s, u_s, o_st):
        g_s[0:8, :] = jnp.zeros((8, D), f32)
        g_s[S + 8:S + 16, :] = jnp.zeros((8, D), f32)

        def load_h(i):
            return h_s[pl.ds(pl.multiple_of(i * bseg, bseg), bseg)].reshape(RB, D)

        def prep(i):
            return _pk(_ln2(load_h(i)).astype(bf16))

        def w1_stage(i):
            a = _upk(a1_s[...])
            r0 = pl.multiple_of(i * RB + 8, 8)
            for c in range(4):
                g = _gelu(_dot(a, _upk(w1_p[:, c * cq:(c + 1) * cq])))
                g_s[pl.ds(r0, RB), c * cq:(c + 1) * cq] = g

        def mix(i):
            r0 = pl.multiple_of(i * RB, RB)
            g0 = g_s[pl.ds(r0, RB + 16), 0 * cq:1 * cq][7:7 + RB]
            g1 = g_s[pl.ds(r0, RB + 16), 1 * cq:2 * cq][9:9 + RB]
            g2 = g_s[pl.ds(r0, RB + 16), 2 * cq:3 * cq][6:6 + RB]
            g3 = g_s[pl.ds(r0, RB + 16), 3 * cq:4 * cq][10:10 + RB]
            gs = jnp.concatenate([g0, g1, g2, g3], axis=1).astype(bf16)
            hsft = _dot(gs, _upk(w2_p[...]))
            hb = load_h(i)
            x1 = _ln(hb) + hsft
            a_s[...] = _pk(_ln(x1).astype(bf16))
            r_s[i % 2] = hb + x1

        def cp_out(i, slot):
            r0 = pl.multiple_of(i * RB, RB)
            return pltpu.make_async_copy(o_st.at[slot], out_hbm.at[pl.ds(r0, RB), :],
                                         sems.at[S_OUT + slot])

        def block(i, slot, with_prep, with_w1, with_mix):
            if with_w1:
                w1_stage(i + 2)
            if with_prep:
                a1_s[...] = prep(i + 3)
            a = _upk(a_s[...])
            for c in range(F // FC):
                u = _dot(a, _upk(w3_p[:, c * FC:(c + 1) * FC]))
                u_s[:, c * FC:(c + 1) * FC] = _pk(_gelu(u).astype(bf16))
            if with_mix:
                mix(i + 1)
            y = _dot(_upk(u_s[...]), _upk(w4_p[...]))
            o_st[slot] = (r_s[slot] + y).astype(bf16)
            cp_out(i, slot).start()

        a1_s[...] = prep(0)
        w1_stage(0)
        a1_s[...] = prep(1)
        w1_stage(1)
        a1_s[...] = prep(2)
        mix(0)

        def body(i, carry, **kw):
            slot = i % 2

            @pl.when(i >= 2)
            def _():
                cp_out(i - 2, slot).wait()

            block(i, slot, **kw)
            return carry

        lax.fori_loop(0, NB - 3, functools.partial(body, with_prep=True, with_w1=True, with_mix=True), 0)
        for i in range(NB - 3, NB):
            cp_out(i - 2, i % 2).wait()
            block(i, i % 2, with_prep=False, with_w1=i + 2 < NB, with_mix=i + 1 < NB)
        cp_out(NB - 2, (NB - 2) % 2).wait()
        cp_out(NB - 1, (NB - 1) % 2).wait()

    pl.run_scoped(
        phase_b,
        pltpu.VMEM((S + 16, D), f32),
        pltpu.VMEM((RB // 2, D), u32),
        pltpu.VMEM((RB // 2, D), u32),
        pltpu.VMEM((2, RB, D), f32),
        pltpu.VMEM((RB // 2, F), u32),
        pltpu.VMEM((2, RB, D), bf16),
    )


@functools.partial(jax.jit, static_argnames=("SEG",))
def _forward(x, mem0, wq, wk, wv, wo, w1, w2, w3, w4, *, SEG):
    B, S, D = x.shape
    _, H, E = wq.shape
    M = mem0.shape[1]
    F = w3.shape[1]
    NSEG = S // SEG
    assert B == 1 and M == 8 and SEG == 32 and E == 128 and S == NSEG * SEG
    assert D == HG * E and H % HG == 0 and H // HG >= 2 and H % 16 == 0
    assert S % RB == 0 and S // RB >= 4 and F % FC == 0
    assert (NSEG * NX) % 256 == 0 and NSEG % 32 == 0
    assert D % (8 * NSEG) == 0 and F % (8 * NSEG) == 0

    hbm = pl.BlockSpec(memory_space=pl.ANY)
    kernel = functools.partial(_kernel, NSEG=NSEG, SEG=SEG, D=D, H=H, E=E, M=M, F=F)
    out = pl.pallas_call(
        kernel,
        out_shape=jax.ShapeDtypeStruct((S, D), x.dtype),
        in_specs=[hbm] * 10,
        out_specs=hbm,
        scratch_shapes=[
            pltpu.VMEM((NSEG, SEG, D), bf16),
            pltpu.VMEM((NSEG, SEG, D), f32),
            pltpu.VMEM((M, D), bf16),
            pltpu.VMEM((D, D), bf16),
            pltpu.VMEM((D, D), bf16),
            pltpu.VMEM((D, F), bf16),
            pltpu.VMEM((F, D), bf16),
            pltpu.VMEM((D // 2, D), u32),
            pltpu.VMEM((D // 2, D), u32),
            pltpu.VMEM((D // 2, F), u32),
            pltpu.VMEM((F // 2, D), u32),
            pltpu.SemaphoreType.DMA((N_SEMS,)),
        ],
        compiler_params=pltpu.CompilerParams(vmem_limit_bytes=124 * 1024 * 1024),
        name="rmt_mixer",
    )(
        x.reshape(NSEG, SEG, D),
        mem0.reshape(M, D),
        wq, wk, wv,
        wo.reshape(H * E, D),
        w1, w2, w3, w4,
    )
    return out.reshape(B, S, D)


def pallas_sequential_preLN__memory_aug_recurrent_mem_tr__mixer_s_mlp__prompt_kernel(
    A_x, A_mem0, A_Wq, A_Wk, A_Wv, A_Wo, A_seg_len, B_x, B_w1, B_w2, B_w3, B_w4
):
    del B_x
    seg = A_seg_len if isinstance(A_seg_len, int) else 32
    return _forward(A_x, A_mem0, A_Wq, A_Wk, A_Wv, A_Wo, B_w1, B_w2, B_w3, B_w4, SEG=seg)
```
